```python
import os as _os
_os.environ.setdefault('JAX_PLATFORMS', 'cpu')
import jax
import jax.numpy as jnp

def _softmax(x, axis=-1):
    return jax.nn.softmax(x, axis=axis)

def _gelu(x):
    return jax.nn.gelu(x, approximate=True)

def _silu(x):
    return jax.nn.silu(x)

def _sigmoid(x):
    return jax.nn.sigmoid(x)

def _layernorm(x, axis=-1, eps=1e-05):
    m = jnp.mean(x, axis=axis, keepdims=True)
    v = jnp.var(x, axis=axis, keepdims=True)
    return (x - m) / jnp.sqrt(v + eps)

def _scatter_add(tgt, idx, src, axis=0):
    return tgt.at[idx].add(src)

def _segment_sum(src, seg, n):
    return jax.ops.segment_sum(src, seg, n)

class _Rng:

    def __init__(self, key):
        self._k = key

    def _next(self):
        self._k, sub = jax.random.split(self._k)
        return sub

    def normal(self, shape):
        return jax.random.normal(self._next(), shape, dtype=jnp.bfloat16)

    def randint(self, lo, hi, shape):
        return jax.random.randint(self._next(), shape, lo, hi, dtype=jnp.int32)

    def uniform(self, shape, lo=0.0, hi=1.0):
        return jax.random.uniform(self._next(), shape, jnp.bfloat16, lo, hi)

    def permutation(self, n):
        return jax.random.permutation(self._next(), n)
kernel_name = 'adaLN_cond__sliding_local_dilated__glu_gated_swiglu__prompt'

def setup_inputs():
    _rng = _Rng(jax.random.key(int.from_bytes(__import__("os").urandom(4), "little")))
    _w = lambda a: (lambda t: t.astype(jnp.bfloat16) if jnp.issubdtype(t.dtype, jnp.floating) else t)(jnp.asarray(a))

    def _A_setup():
        B, S, D = (1, 2048, 576)
        return {'x': _w((lambda *s: _rng.normal(s) * 0.05)(B, S, D)), 'wqkv': _w((lambda *s: _rng.normal(s) * 0.05)(D, 3 * D)), 'wo': _w((lambda *s: _rng.normal(s) * 0.05)(D, D))}
    _A_in = _A_setup()

    def _B_setup():
        B, S, D, F = (1, 2048, 576, 4608)
        return {'x': _w((lambda *s: _rng.normal(s) * 0.05)(B, S, D)), 'w1': _w((lambda *s: _rng.normal(s) * 0.8)(D, F) * (2.0 / D) ** 0.5), 'w3': _w((lambda *s: _rng.normal(s) * 0.8)(D, F) * (2.0 / D) ** 0.5), 'w2': _w((lambda *s: _rng.normal(s) * 0.8)(F, D) * (2.0 / F) ** 0.5)}
    _B_in = _B_setup()
    return {'A_x': _A_in['x'], 'A_wqkv': _A_in['wqkv'], 'A_wo': _A_in['wo'], 'B_x': _B_in['x'], 'B_w1': _B_in['w1'], 'B_w3': _B_in['w3'], 'B_w2': _B_in['w2'], 'c': _w((lambda *s: _rng.normal(s) * 0.05)(1, 576) * 8.0), 'w_mod': _w((lambda *s: _rng.normal(s) * 0.05)(576, 6 * 576) * 576 ** (-0.5) * 8.0)}

def reference(A_x, A_wqkv, A_wo, B_x, B_w1, B_w3, B_w2, c, w_mod):

    def _A_ref(x, wqkv, wo):
        B, S, D = x.shape
        H = 32
        Dh = D // H
        W, dil = (8, 2)
        qkv = (lambda x, *d: x.transpose(*d))((x @ wqkv).reshape(B, S, 3, H, Dh), 2, 0, 3, 1, 4)
        q, k, v = (qkv[0], qkv[1], qkv[2])
        scale = Dh ** (-0.5)
        pos = jnp.arange(S)
        off = jnp.arange(W) * dil
        idx = pos[:, None] - off[None, :]
        mask = idx >= 0
        idx_c = jnp.where(mask, idx, 0).reshape(-1)
        kg = k[:, :, idx_c, :].reshape(B, H, S, W, Dh)
        vg = v[:, :, idx_c, :].reshape(B, H, S, W, Dh)
        logits = jnp.einsum('bhsd,bhswd->bhsw', q, kg) * scale
        logits = jnp.where(mask[None, None, :, :], logits, -1000000000.0)
        attn = _softmax(logits, axis=-1)
        o = jnp.einsum('bhsw,bhswd->bhsd', attn, vg)
        return (lambda x, *d: x.transpose(*d))(o, 0, 2, 1, 3).reshape(B, S, D) @ wo

    def _B_ref(x, w1, w3, w2):
        gate = jnp.einsum('bsd,df->bsf', x, w1)
        up = jnp.einsum('bsd,df->bsf', x, w3)
        h = _silu(gate) * up
        out = jnp.einsum('bsf,fd->bsd', h, w2)
        return out
    x = A_x
    mod = (_silu(c) @ w_mod).reshape(c.shape[0], 6, 1, -1)
    sa, ca, ga, sb, cb, gb = (mod[:, 0].copy(), mod[:, 1].copy(), mod[:, 2].copy(), mod[:, 3].copy(), mod[:, 4].copy(), mod[:, 5].copy())
    h = _layernorm(x, axis=-1) * (1 + ca) + sa
    x = x + ga * _A_ref(h, A_wqkv, A_wo)
    h = _layernorm(x, axis=-1) * (1 + cb) + sb
    x = x + gb * _B_ref(h, B_w1, B_w3, B_w2)
    return x
```

```python
import contextlib
import jax
import jax.numpy as jnp
import jax.experimental.pallas as pl
import jax.experimental.pallas.tpu as pltpu

S, D, F, H, DH, W, DIL = 2048, 576, 4608, 32, 18, 8, 2
f32 = jnp.float32
bf16 = jnp.bfloat16
u32 = jnp.uint32
NT = (((1,), (1,)), ((), ()))
L = 128
TA = 256
NA = S // TA
HD = D // 2
KS = (256, 320, 320, 256, 256, 384, 320)
AOFF = (0, 256, 640, 1024, 1280, 1536, 1920)
AW = 2304
BOFF = {0: 0, 2: 256, 3: 576, 5: 832, 6: 1216}
BROWS = 1536


def _lnT(x):
    m = jnp.mean(x, axis=0, keepdims=True)
    xc = x - m
    v = jnp.mean(xc * xc, axis=0, keepdims=True)
    return xc * jax.lax.rsqrt(v + 1e-5)


def _silu_mul(g, u):
    hg = 0.5 * g
    return (hg * jnp.tanh(hg) + hg) * u


def _sa(x11, x12, x21, x22):
    return [x11 + x22, x21 + x22, x11, x22, x11 + x12, x21 - x11, x12 - x22]


def _sb(y11, y12, y21, y22):
    return [y11 + y22, y11, y12 - y22, y21 - y11, y22, y11 + y12, y21 + y22]


def _pk(v):
    return pltpu.bitcast(v.astype(bf16), u32)


def _upk(v):
    return pltpu.bitcast(v, bf16)


def make(tf=512, mb=422, hg=8, prof=0, order=0, nq=2, no=2, nw=128, rc=64):
    nf = F // tf
    hf = tf // 2
    sizes = [int(ch) * 128 for ch in str(mb)]
    assert sum(sizes) == S // 2
    units = [(sum(sizes[:i]), sizes[i]) for i in range(len(sizes))]
    nsup = len(units)
    nnt = hf // nw
    OORD = (4, 1, 0, 3, 2, 6, 5)
    SOUT = ((((0, 0), 1), ((1, 1), 1)), (((1, 0), 1), ((1, 1), -1)), (((0, 1), 1), ((1, 1), 1)),
            (((0, 0), 1), ((1, 0), 1)), (((0, 0), -1), ((0, 1), 1)), (((1, 1), 1),), (((0, 0), 1),))
    scope = jax.named_scope if prof else (lambda name: contextlib.nullcontext())

    def kernel(x_hbm, c_ref, wmod_hbm, wqkv_hbm, wo_hbm, w1_hbm, w3_hbm, w2t_hbm, out_hbm,
               x_v, wmod_v, wqkv_v, wqkvT, wo_v, woT, w1_v, w3_v, w2t_v,
               modb, h_sc, q_sc, kv_sc, o_sc, x1_sc, a_sc, t_sc, acc, out_v,
               sem_x, sem_w, sem_f, sem_o):
        def cp_x(i):
            return pltpu.make_async_copy(x_hbm.at[:, pl.ds(i * TA, TA)], x_v.at[i], sem_x.at[i])

        def cp_f(k, j):
            src, dst = ((w1_hbm, w1_v), (w3_hbm, w3_v), (w2t_hbm, w2t_v))[k]
            return pltpu.make_async_copy(src.at[:, pl.ds(j * tf, tf)], dst.at[j], sem_f.at[k, j])

        cp_wqkv = pltpu.make_async_copy(wqkv_hbm, wqkv_v, sem_w.at[0])
        cp_moda = pltpu.make_async_copy(wmod_hbm.at[:, pl.ds(0, 1152)], wmod_v.at[:, pl.ds(0, 1152)], sem_w.at[1])
        cp_modb = pltpu.make_async_copy(wmod_hbm.at[:, pl.ds(1152, 2304)], wmod_v.at[:, pl.ds(1152, 2304)], sem_w.at[2])
        cp_wo = pltpu.make_async_copy(wo_hbm, wo_v, sem_w.at[3])

        cp_wqkv.start()
        cp_x(0).start()
        cp_moda.start()

        acc[...] = jnp.zeros(acc.shape, f32)
        kv_sc[0] = jnp.zeros(kv_sc.shape[1:], u32)

        c = c_ref[...].astype(f32)
        sc = jnp.broadcast_to((c * jax.nn.sigmoid(c)).astype(bf16), (16, D))

        def mod_part(lo, n):
            mod = jnp.dot(sc, wmod_v[:, lo * D:(lo + n) * D], preferred_element_type=f32)
            for j in range(n):
                row = mod[0:1, j * D:(j + 1) * D]
                if (lo + j) % 3 == 1:
                    row = row + 1.0
                modb[lo + j] = jnp.broadcast_to(row, (L, D)).T

        GR = 3 * hg * DH
        HR = hg * DH
        ng = H // hg

        def ln1(i, sl):
            hs = []
            for t in range(2):
                x = x_v[i, :, t * L:(t + 1) * L].astype(f32)
                hs.append(_lnT(x) * modb[1] + modb[0])
            h_sc[sl] = jnp.concatenate(hs, axis=1).astype(bf16)

        def qkv_part(i, u):
            res = jnp.dot(pltpu.bitcast(wqkvT[u * GR // 2:(u + 1) * GR // 2, :], bf16), h_sc[i % 2],
                          preferred_element_type=f32)
            for t in range(2):
                q_sc[t, u] = res[0:HR, t * L:(t + 1) * L]
                kv_sc[2 * i + t + 1, u] = pltpu.bitcast(res[HR:GR, t * L:(t + 1) * L].astype(bf16), u32)

        def unpack(wd):
            lo = pltpu.bitcast(wd << 16, f32)
            hi = pltpu.bitcast(wd & jnp.uint32(0xFFFF0000), f32)
            return lo, hi

        def attn(i, u):
            slot = i % 2
            lane = jax.lax.broadcasted_iota(jnp.int32, (hg, L), 1)
            for t in range(2):
                g = 2 * i + t
                pos = lane + g * L

                def shifted(base, p):
                    cur = kv_sc[g + 1, u, pl.ds(base + p, hg, stride=9), :]
                    prev = kv_sc[g, u, pl.ds(base + p, hg, stride=9), :]
                    res = [cur]
                    for w in range(1, W):
                        res.append(pltpu.roll(jnp.where(lane < L - DIL * w, cur, prev), DIL * w, 1))
                    return res

                lg = [None] * W
                for p in range(9):
                    q0 = q_sc[t, u, pl.ds(2 * p, hg, stride=DH), :]
                    q1 = q_sc[t, u, pl.ds(2 * p + 1, hg, stride=DH), :]
                    ks = shifted(0, p)
                    for w in range(W):
                        lo, hi = unpack(ks[w])
                        tmp = q0 * lo + q1 * hi
                        lg[w] = tmp if lg[w] is None else lg[w] + tmp
                lg = [l * (DH ** -0.5) for l in lg]
                for w in range(1, W):
                    lg[w] = jnp.where(pos >= DIL * w, lg[w], -1e9)
                m = lg[0]
                for w in range(1, W):
                    m = jnp.maximum(m, lg[w])
                es = [jnp.exp(l - m) for l in lg]
                den = es[0]
                for w in range(1, W):
                    den = den + es[w]
                inv = 1.0 / den
                at = [e * inv for e in es]
                for p in range(9):
                    vs = shifted(HR // 2, p)
                    o0 = o1 = None
                    for w in range(W):
                        lo, hi = unpack(vs[w])
                        o0 = at[w] * lo if o0 is None else o0 + at[w] * lo
                        o1 = at[w] * hi if o1 is None else o1 + at[w] * hi
                    o_sc[slot, t, pl.ds(u * HR + 2 * p, hg, stride=DH), :] = o0
                    o_sc[slot, t, pl.ds(u * HR + 2 * p + 1, hg, stride=DH), :] = o1

        def wo_res(i):
            slot = i % 2
            o = jnp.concatenate([o_sc[slot, 0], o_sc[slot, 1]], axis=1).astype(bf16)
            mo = D // no
            for r in range(no):
                att = jnp.dot(pltpu.bitcast(woT[r * mo // 2:(r + 1) * mo // 2, :], bf16), o, preferred_element_type=f32)
                rs = slice(r * mo, (r + 1) * mo)
                for t in range(2):
                    x1_sc[2 * i + t, rs] = (x_v[i, rs, t * L:(t + 1) * L].astype(f32)
                                            + modb[2, rs] * att[:, t * L:(t + 1) * L])

        def ln2(i):
            h2 = [(_lnT(x1_sc[2 * i + t]) * modb[4] + modb[3]).T for t in range(2)]
            r0 = i * 32 if isinstance(i, int) else pl.multiple_of(i * 32, 32)
            lv1 = _sa(h2[0][:, 0:256], h2[0][:, 256:512], h2[1][:, 0:256], h2[1][:, 256:512])
            for a in range(7):
                x = lv1[a]
                lv2 = _sa(x[0:64, 0:L], x[0:64, L:], x[64:, 0:L], x[64:, L:])
                for b in range(7):
                    a_sc[7 * a + b, pl.ds(r0, 32), :] = _pk(lv2[b])
            for t in range(2):
                for a2 in range(2):
                    t_sc[2 * t + a2, pl.ds(r0, 32), :] = _pk(h2[t][64 * a2:64 * a2 + 64, 512:576])

        x1_sc[0:2] = jnp.zeros((2, D, L), f32)
        with scope("w_wqkv"):
            cp_wqkv.wait()
        with scope("tr_wqkv"):
            wt = pltpu.bitcast(wqkv_v[...].T, u32)
            for part in range(3):
                for u in range(ng):
                    src = (part * D + u * HR) // 2
                    dst = (u * GR + part * HR) // 2
                    wqkvT[dst:dst + HR // 2, :] = wt[src:src + HR // 2, :]
        with scope("w_moda"):
            cp_moda.wait()
            cp_x(0).wait()
        cp_x(1).start()
        cp_wo.start()
        cp_modb.start()
        with scope("a_0a"):
            mod_part(0, 2)
            ln1(0, 0)
            for u in range(ng):
                qkv_part(0, u)
                if u > 0:
                    attn(0, u - 1)
        with scope("w_2"):
            cp_x(1).wait()
            cp_wo.wait()
            cp_modb.wait()
        for i in range(2, NA):
            cp_x(i).start()
        with scope("a_0b"):
            attn(0, ng - 1)
            ln1(1, 1)
            woT[...] = pltpu.bitcast(wo_v[...].T, u32)
            mod_part(2, 4)

        def a_body(i, carry):
            nx = jnp.minimum(i + 1, NA - 1)
            with scope("w_x"):
                @pl.when(i + 1 < NA)
                def _():
                    cp_x(nx).wait()
            for k in range(3):
                cp_f(k, i - 1).start()
            with scope("a_body"):
                if order == 0:
                    qkv_part(i, 0)
                    ln2(jnp.maximum(i - 2, 0))
                    for u in range(1, ng):
                        qkv_part(i, u)
                        attn(i, u - 1)
                    wo_res(i - 1)
                    attn(i, ng - 1)
                    ln1(nx, (i + 1) % 2)
                elif order == 1:
                    ln2(jnp.maximum(i - 2, 0))
                    for u in range(ng):
                        qkv_part(i, u)
                    wo_res(i - 1)
                    for u in range(ng):
                        attn(i, u)
                    ln1(nx, (i + 1) % 2)
                elif order == 2:
                    qkv_part(i, 0)
                    ln2(jnp.maximum(i - 2, 0))
                    ln1(nx, (i + 1) % 2)
                    for u in range(1, ng):
                        qkv_part(i, u)
                        attn(i, u - 1)
                    wo_res(i - 1)
                    attn(i, ng - 1)
            return carry

        jax.lax.fori_loop(1, NA, a_body, 0)
        for j in range(NA - 1, nf):
            for k in range(3):
                cp_f(k, j).start()
        with scope("a_epi"):
            wo_res(NA - 1)
            ln2(NA - 2)
            ln2(NA - 1)

        def cp_o(i):
            return pltpu.make_async_copy(out_v.at[i], out_hbm.at[:, pl.ds(i * TA, TA)], sem_o.at[i])

        def fin(i):
            cs = slice(i * L, (i + 1) * L)
            m = [acc[k, :, cs] for k in range(7)]
            gb = modb[5]
            out_v[i, 0:HD, 0:L] = (x1_sc[2 * i, 0:HD] + gb[0:HD] * (m[0] + m[3] - m[4] + m[6])).astype(bf16)
            out_v[i, 0:HD, L:2 * L] = (x1_sc[2 * i + 1, 0:HD] + gb[0:HD] * (m[2] + m[4])).astype(bf16)
            out_v[i, HD:D, 0:L] = (x1_sc[2 * i, HD:D] + gb[HD:D] * (m[1] + m[3])).astype(bf16)
            out_v[i, HD:D, L:2 * L] = (x1_sc[2 * i + 1, HD:D] + gb[HD:D] * (m[0] - m[1] + m[2] + m[5])).astype(bf16)

        n_early = units[-1][0] // L

        def b_body(j, carry):
            with scope("w_f"):
                for k in range(3):
                    cp_f(k, j).wait()
            lv1 = _sb(w1_v[j, 0:256, :].astype(f32), w3_v[j, 0:256, :].astype(f32),
                      w1_v[j, 256:512, :].astype(f32), w3_v[j, 256:512, :].astype(f32))
            bw = {}
            for a in OORD:
                y = lv1[a]
                lv2 = _sb(y[0:L, 0:hf], y[0:L, hf:], y[L:, 0:hf], y[L:, hf:])
                for b in range(7):
                    for nn in range(nnt):
                        bw[(a, b, nn)] = lv2[b][:, nn * nw:(nn + 1) * nw].astype(bf16)
            c11 = w2t_v[j, 0:HD, 0:hf].astype(f32)
            c12 = w2t_v[j, 0:HD, hf:tf].astype(f32)
            c21 = w2t_v[j, HD:D, 0:hf].astype(f32)
            c22 = w2t_v[j, HD:D, hf:tf].astype(f32)
            aw = [v.astype(bf16) for v in _sa(c11, c12, c21, c22)]

            def aop(i):
                return aw[i]

            QS = ((0, 0), (0, 1), (1, 0), (1, 1))

            def gu(tt):
                st, sz = units[tt]
                rq = slice(st // 4, (st + sz) // 4)
                prods = {}
                for nn in range(nnt):
                    cs = slice(nn * nw, (nn + 1) * nw)
                    for a in OORD:
                        for b in OORD:
                            prods[(nn, a, b)] = jnp.dot(_upk(a_sc[7 * a + b, rq, :]), bw[(a, b, nn)],
                                                        preferred_element_type=f32)
                    for a1 in range(2):
                        for a2 in range(2):
                            for c1 in range(2):
                                for c2 in range(2):
                                    wv = (w1_v, w3_v)[c1]
                                    col = c2 * hf + nn * nw
                                    prods[(nn, 't', a1, a2, c1, c2)] = jnp.dot(
                                        _upk(t_sc[2 * a1 + a2, rq, :]), wv[j, 512:576, col:col + nw],
                                        preferred_element_type=f32)
                return prods

            def combine(tt, prods):
                mq = units[tt][1] // 2
                pieces = {}
                for nn in range(nnt):
                    for r in range(mq // rc):
                        sl = slice(r * rc, (r + 1) * rc)
                        cacc = {}
                        for a1, c1 in QS:
                            for a2, c2 in QS:
                                cacc[(a1, c1, a2, c2)] = prods[(nn, 't', a1, a2, c1, c2)][sl]
                        for a in range(7):
                            p = [prods[(nn, a, b)][sl] for b in range(7)]
                            inn = {(0, 0): p[0] + p[3] - p[4] + p[6], (0, 1): p[2] + p[4],
                                   (1, 0): p[1] + p[3], (1, 1): p[0] - p[1] + p[2] + p[5]}
                            for tgt, sign in SOUT[a]:
                                for q in QS:
                                    key = tgt + q
                                    cacc[key] = cacc[key] + inn[q] if sign > 0 else cacc[key] - inn[q]
                        for a2 in range(2):
                            e = {(a1, c2): _silu_mul(cacc[(a1, 0, a2, c2)], cacc[(a1, 1, a2, c2)])
                                 for a1 in range(2) for c2 in range(2)}
                            eb = _sb(e[(0, 0)], e[(1, 0)], e[(0, 1)], e[(1, 1)])
                            for i in range(7):
                                pieces[(i, nn, a2, r)] = eb[i]
                out = []
                per = 64 // rc
                for i in range(7):
                    cols = []
                    for nn in range(nnt):
                        rows = []
                        for tl in range(mq // 64):
                            for a2 in range(2):
                                for rr in range(per):
                                    rows.append(pieces[(i, nn, a2, tl * per + rr)])
                        cols.append(jnp.concatenate(rows, axis=0))
                    out.append(jnp.concatenate(cols, axis=1).astype(bf16))
                return out

            def down(tt, eb):
                st, sz = units[tt]
                rs = slice(st, st + sz)
                for i in range(7):
                    acc[i, :, rs] += jax.lax.dot_general(aop(i), eb[i], NT, preferred_element_type=f32)

            pr = gu(0)
            for tt in range(nsup):
                prn = gu(tt + 1) if tt + 1 < nsup else None
                down(tt, combine(tt, pr))
                pr = prn
                if tt + 1 < nsup:
                    tiles = range(units[tt][0] // L, (units[tt][0] + units[tt][1]) // L)
                    for i in tiles:
                        fin(i)

                    @pl.when(j == nf - 1)
                    def _():
                        for i in tiles:
                            cp_o(i).start()
            return carry

        with scope("b_loop"):
            jax.lax.fori_loop(0, nf, b_body, 0)

        with scope("fin"):
            for i in range(n_early, NA):
                fin(i)
                cp_o(i).start()
        with scope("w_out"):
            for i in range(NA):
                cp_o(i).wait()

    def fn(A_x, A_wqkv, A_wo, B_x, B_w1, B_w3, B_w2, c, w_mod):
        xT = A_x.reshape(S, D).T
        w2t = B_w2.T
        hbm = pl.BlockSpec(memory_space=pl.ANY)
        outT = pl.pallas_call(
            kernel,
            in_specs=[hbm, pl.BlockSpec(memory_space=pltpu.VMEM), hbm, hbm, hbm, hbm, hbm, hbm],
            out_specs=hbm,
            out_shape=jax.ShapeDtypeStruct((D, S), bf16),
            scratch_shapes=[
                pltpu.VMEM((NA, D, TA), bf16),
                pltpu.VMEM((D, 6 * D), bf16),
                pltpu.VMEM((D, 3 * D), bf16),
                pltpu.VMEM((3 * D // 2, D), u32),
                pltpu.VMEM((D, D), bf16),
                pltpu.VMEM((D // 2, D), u32),
                pltpu.VMEM((nf, D, tf), bf16),
                pltpu.VMEM((nf, D, tf), bf16),
                pltpu.VMEM((nf, D, tf), bf16),
                pltpu.VMEM((6, D, L), f32),
                pltpu.VMEM((2, D, TA), bf16),
                pltpu.VMEM((2, H // hg, hg * DH, L), f32),
                pltpu.VMEM((2 * NA + 1, H // hg, hg * DH, L), u32),
                pltpu.VMEM((2, 2, D, L), f32),
                pltpu.VMEM((2 * NA, D, L), f32),
                pltpu.VMEM((49, S // 8, L), u32),
                pltpu.VMEM((4, S // 8, 64), u32),
                pltpu.VMEM((7, HD, S // 2), f32),
                pltpu.VMEM((NA, D, TA), bf16),
                pltpu.SemaphoreType.DMA((NA,)),
                pltpu.SemaphoreType.DMA((4,)),
                pltpu.SemaphoreType.DMA((3, nf)),
                pltpu.SemaphoreType.DMA((NA,)),
            ],
            compiler_params=pltpu.CompilerParams(vmem_limit_bytes=100 * 1024 * 1024),
        )(xT, c, w_mod, A_wqkv, A_wo, B_w1, B_w3, w2t)
        return outT.T.reshape(1, S, D)

    return fn


pallas_adaLN_cond__sliding_local_dilated__glu_gated_swiglu__prompt_kernel = jax.jit(make())
```

```python
import contextlib
import jax
import jax.numpy as jnp
import jax.experimental.pallas as pl
import jax.experimental.pallas.tpu as pltpu

S, D, F, H, DH, W, DIL = 2048, 576, 4608, 32, 18, 8, 2
f32 = jnp.float32
bf16 = jnp.bfloat16
u32 = jnp.uint32
NT = (((1,), (1,)), ((), ()))
L = 128
TA = 256
NA = S // TA
HD = D // 2
KS = (256, 320, 320, 256, 256, 384, 320)
AOFF = (0, 256, 640, 1024, 1280, 1536, 1920)
AW = 2304
BOFF = {0: 0, 2: 256, 3: 576, 5: 832, 6: 1216}
BROWS = 1536


class _Ticker:
    def __init__(self, toks, n=1):
        self.toks, self.n, self.k = toks, n, 0

    def __call__(self):
        if not self.toks:
            return None
        tok = self.toks[min(self.k * len(self.toks) // self.n, len(self.toks) - 1)]
        self.k += 1
        return jnp.where(tok > jnp.inf, 1.0, 0.0)


def _sel(toks, spec):
    out = []
    for part in str(spec).split('_'):
        if '-' in part:
            lo, hi = part.split('-')
            out += toks[int(lo):int(hi)]
    return out


def _toks(res):
    return [res[r:r + 8, t * L:(t + 1) * L] for t in range(res.shape[1] // L) for r in range(0, res.shape[0], 8)]


class _Idx:
    def __init__(self, base, off=0):
        self.base, self.off = base, off

    def __add__(self, k):
        return _Idx(self.base, self.off + k)

    def __sub__(self, k):
        return _Idx(self.base, self.off - k)

    def __mod__(self, m):
        assert m == 2
        return self.off % 2

    def __rmul__(self, k):
        return k * self.base + k * self.off

    __mul__ = __rmul__

    @property
    def v(self):
        return self.base + self.off


def _iv(i):
    return i.v if isinstance(i, _Idx) else i


def _plus(v, tick):
    if tick is None:
        return v
    n = v.shape[1] // L
    return v + (tick if n == 1 else jnp.concatenate([tick] * n, axis=1))


def _stats(k8, s1, s2):
    md = jnp.sum(s1, axis=0, keepdims=True) * (1.0 / D)
    var = jnp.sum(s2, axis=0, keepdims=True) * (1.0 / D) - md * md
    rs = jax.lax.rsqrt(jnp.maximum(var, 0.0) + 1e-5)
    return k8 + md, jnp.broadcast_to(rs, k8.shape)


def _silu_mul(g, u):
    hg = 0.5 * g
    return (hg * jnp.tanh(hg) + hg) * u


def _sa(x11, x12, x21, x22):
    return [x11 + x22, x21 + x22, x11, x22, x11 + x12, x21 - x11, x12 - x22]


def _sb(y11, y12, y21, y22):
    return [y11 + y22, y11, y12 - y22, y21 - y11, y22, y11 + y12, y21 + y22]


LAM = (-2.0, -0.5, 0.5, 2.0)
PAIRS = tuple((i, j) for i in range(4) for j in range(i + 1, 4))


def _hk_a(x, y):
    z = [[y[i] + LAM[l] * x[i] for i in range(4)] for l in range(4)]
    ops = [x[i] for i in range(4)] + [z[i][i] for i in range(4)]
    for i, j in PAIRS:
        r = 1.0 / (LAM[i] - LAM[j])
        ops += [(z[i][i] - z[j][j]) * r, (z[j][i] - z[j][j]) * r, (z[i][j] - z[i][i]) * r]
    return ops


def _hk_b(b1, b2):
    sub = lambda v, l, j: v - LAM[l] * b2[j]
    u = [sub(b1[i], i, i) for i in range(4)]
    ops = u + list(b2)
    for i, j in PAIRS:
        ops += [u[i] + u[j], sub(u[i] + b1[j], i, j), sub(u[j] + b1[i], j, i)]
    return ops


def _hk_c_row(m, i, tick=None):
    p = m(i) if tick is None else m(i) + tick
    out = []
    for j in range(4):
        if j == i:
            out.append(p + m(4 + i))
        else:
            k = 8 + 3 * PAIRS.index((min(i, j), max(i, j)))
            v = (m(4 + j) - p) + m(k)
            out.append(v - m(k + 1) if i < j else v + m(k + 2))
    return out


def _pack2(a, b):
    half = jnp.uint32(0x8000)
    lo = (pltpu.bitcast(a, u32) + half) >> 16
    hi = (pltpu.bitcast(b, u32) + half - lo) & jnp.uint32(0xFFFF0000)
    return hi | lo


def _pk(v):
    return pltpu.bitcast(v.astype(bf16), u32)


def _upk(v):
    return pltpu.bitcast(v, bf16)


def make(tf=512, mb=422, hg=8, prof=0, no=2, gord=1, fr=16, fpace=1, dofin=1, nofuse=1, dord=1, fst=1, ga=4, gb_=88, da=2, db=22, c1=16, c2=48, c3=16, nq=3, t1='216-560', t2a='0', t2b='40-108_490-570', te='0-100', tp1='0-150', kvm=0, skipb=0, aun=2, xp=0, apl=0, pb=3, mcut='0x5x8x11'):
    nf = F // tf
    hf = tf // 2
    sizes = [int(ch) * 128 for ch in str(mb)]
    assert sum(sizes) == S // 2
    units = [(sum(sizes[:i]), sizes[i]) for i in range(len(sizes))]
    nsup = len(units)
    QD = D // 4
    DORD = list(range(26)) if dord == 0 else [4, 5, 6, 7, 0, 1, 2, 3] + list(range(8, 26)) if dord == 2 else [0, 9, 12, 15, 4, 1, 8, 10, 18, 21, 5, 2, 11, 13, 17, 19, 24, 6, 3, 14, 16, 20, 22, 23, 25, 7] if dord == 3 else [4, 0, 5, 1, 8, 9, 10, 6, 2, 11, 12, 13, 17, 18, 19, 7, 3, 14, 15, 16, 20, 21, 22, 23, 24, 25]
    n1 = 2 * (D // c1)
    n2a = 2 * (D // c2)
    n2b = 7 * (64 // c3)
    OORD = (4, 1, 0, 3, 2, 6, 5)
    SOUT = ((((0, 0), 1), ((1, 1), 1)), (((1, 0), 1), ((1, 1), -1)), (((0, 1), 1), ((1, 1), 1)),
            (((0, 0), 1), ((1, 0), 1)), (((0, 0), -1), ((0, 1), 1)), (((1, 1), 1),), (((0, 0), 1),))
    SIN = (((0, 0), (1, 1), 1), ((1, 0), (1, 1), 1), ((0, 0), None, 0), ((1, 1), None, 0),
           ((0, 0), (0, 1), 1), ((1, 0), (0, 0), -1), ((0, 1), (1, 1), -1))
    scope = jax.named_scope if prof else (lambda name: contextlib.nullcontext())

    def kernel(x_hbm, c_hbm, wmod_hbm, wqkv_hbm, wo_hbm, w1_hbm, w3_hbm, w2t_hbm, out_hbm,
               c_v, x_v, wmod_v, wqkv_v, wqkvT, wo_v, woT, w1_v, w3_v, w2t_v,
               modb, modr, h_sc, q_sc, kv_sc, o_sc, x1_sc, st_sc, a_sc, t_sc, acc, out_v,
               sem):
        XSEM = (0, 4, 5, 0, 0, 1, 1, 1)

        def cp_x(i):
            return pltpu.make_async_copy(x_hbm.at[:, pl.ds(i * TA, TA)], x_v.at[i], sem.at[XSEM[i]])

        def cp_f(k, j):
            src, dst = ((w1_hbm, w1_v), (w3_hbm, w3_v), (w2t_hbm, w2t_v))[k]
            return pltpu.make_async_copy(src.at[:, pl.ds(j * tf, tf)], dst.at[j], sem.at[2])

        WQ = ((0, 384), (512, 896), (1152, 1536), (384, 512), (896, 1152), (1536, 1728))

        def cp_wq(k):
            lo, hi = WQ[k]
            return pltpu.make_async_copy(wqkv_hbm.at[:, pl.ds(lo, hi - lo)], wqkv_v.at[:, pl.ds(lo, hi - lo)],
                                         sem.at[min(1 + k, 4)])

        cp_moda = pltpu.make_async_copy(wmod_hbm.at[:, pl.ds(0, 1152)], wmod_v.at[:, pl.ds(0, 1152)], sem.at[0])
        cp_modb = pltpu.make_async_copy(wmod_hbm.at[:, pl.ds(1152, 1792)], wmod_v.at[:, pl.ds(1152, 1792)], sem.at[5])
        cp_modc = pltpu.make_async_copy(wmod_hbm.at[:, pl.ds(2944, 512)], wmod_v.at[:, pl.ds(2944, 512)], sem.at[1])
        cp_c = pltpu.make_async_copy(c_hbm, c_v, sem.at[0])
        cp_wo = pltpu.make_async_copy(wo_hbm, wo_v, sem.at[5])

        cp_moda.start()
        cp_x(0).start()
        cp_c.start()
        for cp in [cp_wq(k) for k in range(6)] + [cp_x(1), cp_wo, cp_modb, cp_x(2)]:
            cp.start(priority=1)

        acc[...] = jnp.zeros(acc.shape, f32)
        kv_sc[0] = jnp.zeros(kv_sc.shape[1:], u32)

        def mod_cols(lo, hi):
            c = c_v[...].astype(f32)
            sc = jnp.broadcast_to((c * jax.nn.sigmoid(c)).astype(bf16), (16, D))
            return jnp.dot(sc, wmod_v[:, lo:hi], preferred_element_type=f32)[0:8]

        def col_bcast(row):
            return jnp.broadcast_to(row[0:1], (L, D)).T

        GR = 3 * hg * DH
        HR = hg * DH
        ng = H // hg

        def ln1(i, i2, sl, tk):
            k8 = jnp.broadcast_to(x_v[i, 0:16, :].astype(f32)[0:1], (8, TA))
            s1 = s2 = None
            for r in range(0, D, 16):
                if r % c1 == 0:
                    kk = _plus(k8, tk())
                x = x_v[i, r:r + 16, :].astype(f32)
                for h in range(2):
                    d = x[8 * h:8 * h + 8] - kk
                    s1 = d if s1 is None else s1 + d
                    s2 = d * d if s2 is None else s2 + d * d
            m8, rs8 = _stats(k8, s1, s2)
            for r in range(0, D, 16):
                if r % c1 == 0:
                    mk = _plus(m8, tk())
                x = x_v[i2, r:r + 16, :].astype(f32)
                for h in range(2):
                    rr = slice(r + 8 * h, r + 8 * h + 8)
                    xn = (x[8 * h:8 * h + 8] - mk) * rs8
                    for t in range(2):
                        h_sc[sl, t, rr] = xn[:, t * L:(t + 1) * L] * modb[1, rr] + modb[0, rr]

        def qkv_part(i, u, hooks=None):
            h = jnp.concatenate([h_sc[i % 2, 0], h_sc[i % 2, 1]], axis=1).astype(bf16)
            toks = []
            mr = GR // nq
            parts = []
            for r in range(nq):
                lo = (u * GR + r * mr) // 2
                parts.append(jnp.dot(pltpu.bitcast(wqkvT[lo:lo + mr // 2, :], bf16), h, preferred_element_type=f32))
                toks += _toks(parts[-1])
                if hooks:
                    hooks.pop(0)()
            res = jnp.concatenate(parts, axis=0)
            for t in range(2):
                q_sc[t, u] = res[0:HR, t * L:(t + 1) * L]
                if kvm:
                    kv_sc[2 * i + t + 1, u] = _pack2(res[HR:2 * HR, t * L:(t + 1) * L], res[2 * HR:GR, t * L:(t + 1) * L])
                else:
                    kv_sc[2 * i + t + 1, u] = pltpu.bitcast(res[HR:GR, t * L:(t + 1) * L].astype(bf16), u32)
            return toks

        def unpack(wd):
            lo = pltpu.bitcast(wd << 16, f32)
            hi = pltpu.bitcast(wd & jnp.uint32(0xFFFF0000), f32)
            return lo, hi

        def attn(i, u):
            slot = i % 2
            lane = jax.lax.broadcasted_iota(jnp.int32, (hg, L), 1)
            for t in range(2):
                g = 2 * i + t
                pos = lane + g * L

                def shifted(base, p):
                    cur = kv_sc[g + 1, u, pl.ds(base + p, hg, stride=9), :]
                    prev = kv_sc[g, u, pl.ds(base + p, hg, stride=9), :]
                    res = [cur]
                    for w in range(1, W):
                        res.append(pltpu.roll(jnp.where(lane < L - DIL * w, cur, prev), DIL * w, 1))
                    return res

                lg = [None] * W
                if kvm:
                    words = []
                    for d in range(DH):
                        cur = kv_sc[g + 1, u, pl.ds(d, hg, stride=DH), :]
                        prev = kv_sc[g, u, pl.ds(d, hg, stride=DH), :]
                        ws = [cur] + [pltpu.roll(jnp.where(lane < L - DIL * w, cur, prev), DIL * w, 1)
                                      for w in range(1, W)]
                        words.append(ws)
                        q0 = q_sc[t, u, pl.ds(d, hg, stride=DH), :]
                        for w in range(W):
                            tmp = q0 * pltpu.bitcast(ws[w] << 16, f32)
                            lg[w] = tmp if lg[w] is None else lg[w] + tmp
                for p in range(0 if kvm else 9):
                    q0 = q_sc[t, u, pl.ds(2 * p, hg, stride=DH), :]
                    q1 = q_sc[t, u, pl.ds(2 * p + 1, hg, stride=DH), :]
                    ks = shifted(0, p)
                    for w in range(W):
                        lo, hi = unpack(ks[w])
                        tmp = q0 * lo + q1 * hi
                        lg[w] = tmp if lg[w] is None else lg[w] + tmp
                lg = [l * (DH ** -0.5) for l in lg]
                for w in range(1, W):
                    lg[w] = jnp.where(pos >= DIL * w, lg[w], -1e9)
                m = lg[0]
                for w in range(1, W):
                    m = jnp.maximum(m, lg[w])
                es = [jnp.exp(l - m) for l in lg]
                den = es[0]
                for w in range(1, W):
                    den = den + es[w]
                inv = 1.0 / den
                at = [e * inv for e in es]
                if kvm:
                    for d in range(DH):
                        o0 = None
                        for w in range(W):
                            tmp = at[w] * pltpu.bitcast(words[d][w], f32)
                            o0 = tmp if o0 is None else o0 + tmp
                        o_sc[slot, t, pl.ds(u * HR + d, hg, stride=DH), :] = o0
                for p in range(0 if kvm else 9):
                    vs = shifted(HR // 2, p)
                    o0 = o1 = None
                    for w in range(W):
                        lo, hi = unpack(vs[w])
                        o0 = at[w] * lo if o0 is None else o0 + at[w] * lo
                        o1 = at[w] * hi if o1 is None else o1 + at[w] * hi
                    o_sc[slot, t, pl.ds(u * HR + 2 * p, hg, stride=DH), :] = o0
                    o_sc[slot, t, pl.ds(u * HR + 2 * p + 1, hg, stride=DH), :] = o1

        def wo_res(i):
            slot = i % 2
            o = jnp.concatenate([o_sc[slot, 0], o_sc[slot, 1]], axis=1).astype(bf16)
            mo = D // no
            k8, s1, s2 = [None] * 2, [None] * 2, [None] * 2
            toks = []
            for r in range(no):
                att = jnp.dot(pltpu.bitcast(woT[r * mo // 2:(r + 1) * mo // 2, :], bf16), o, preferred_element_type=f32)
                toks += _toks(att)
                rs = slice(r * mo, (r + 1) * mo)
                x = x_v[_iv(i), rs, :].astype(f32)
                for t in range(2):
                    x1 = x[:, t * L:(t + 1) * L] + att[:, t * L:(t + 1) * L]
                    x1_sc[2 * i + t, rs] = x1
                    if r == 0:
                        k8[t] = jnp.broadcast_to(x1[0:1], (8, L))
                    for q in range(0, mo, 8):
                        d = x1[q:q + 8] - k8[t]
                        s1[t] = d if s1[t] is None else s1[t] + d
                        s2[t] = d * d if s2[t] is None else s2[t] + d * d
            for t in range(2):
                st_sc[2 * i + t, 0], st_sc[2 * i + t, 1], st_sc[2 * i + t, 2] = k8[t], s1[t], s2[t]
            return toks

        def ln2(i, tk0, tk):
            ln2b(i, ln2a(i, tk0), tk)

        def ln2a(i, tk0):
            h2 = []
            for t in range(2):
                m8, rs8 = _stats(st_sc[2 * i + t, 0], st_sc[2 * i + t, 1], st_sc[2 * i + t, 2])
                rows = []
                for r in range(0, D, 8):
                    if r % c2 == 0:
                        mk = _plus(m8, tk0())
                    rr = slice(r, r + 8)
                    rows.append((x1_sc[2 * i + t, rr] - mk) * rs8)
                h2.append(jnp.concatenate(rows, axis=0).T * modr[1, 0:1] + modr[0, 0:1])
            return h2

        def ln2b(i, h2, tk):
            r0 = i * 32 if isinstance(i, int) else pl.multiple_of(i * 32, 32)
            for t in range(2):
                for a2 in range(2):
                    t_sc[2 * t + a2, pl.ds(r0, 32), :] = _pk(h2[t][64 * a2:64 * a2 + 64, 512:576])
            blk = ((h2[0][:, 0:256], h2[0][:, 256:512]), (h2[1][:, 0:256], h2[1][:, 256:512]))
            for a in (2, 4, 5, 0, 1, 3, 6):
                (p0, p1, sgn) = SIN[a]
                for r in range(0, 64, c3):
                    tick = tk()
                    xs = []
                    for a2 in range(2):
                        rows = []
                        for q in range(64 * a2 + r, 64 * a2 + r + c3, 8):
                            v = _plus(blk[p0[0]][p0[1]][q:q + 8], tick)
                            if p1 is not None:
                                o = blk[p1[0]][p1[1]][q:q + 8]
                                v = v + o if sgn > 0 else v - o
                            rows.append(v)
                        xs.append(jnp.concatenate(rows, axis=0))
                    lv2 = _sa(xs[0][:, 0:L], xs[0][:, L:], xs[1][:, 0:L], xs[1][:, L:])
                    for b in range(7):
                        a_sc[7 * a + b, pl.ds(r0 + r // 2, c3 // 2), :] = _pk(lv2[b])

        notick = _Ticker(None)
        with scope("w_moda"):
            cp_c.wait()
            cp_moda.wait()
            cp_x(0).wait()
        with scope("mod_ln"):
            mod = mod_cols(0, 2 * D)
            modb[0] = col_bcast(mod[:, 0:D])
            modb[1] = col_bcast(mod[:, D:2 * D] + 1.0)
            ln1(0, 0, 0, notick)

        def tr_wq(k):
            lo, hi = WQ[k]
            wt = pltpu.bitcast(wqkv_v[:, lo:hi].T, u32)
            c = lo
            while c < hi:
                e = min(hi, (c // HR + 1) * HR)
                part, u = c // D, (c % D) // HR
                dst = u * GR + part * HR + c % HR
                wqkvT[dst // 2:(dst + e - c) // 2, :] = wt[(c - lo) // 2:(e - lo) // 2, :]
                c = e

        with scope("tr_wqkv"):
            for k in range(2):
                cp_wq(k).wait()
                tr_wq(k)
        with scope("w_wq2"):
            cp_wq(2).wait()
        with scope("a_0a"):
            tr_wq(2)
            qkv_part(0, 0)
            qkv_part(0, 1)
            attn(0, 0)
        with scope("w_wqb"):
            for k in range(3, 6):
                cp_wq(k).wait()
            cp_x(1).wait()
        with scope("a_0"):
            for k in range(3, 6):
                tr_wq(k)
            toks = []
            for u in range(2, ng):
                toks += qkv_part(0, u)
                attn(0, u - 1)
            ln1(1, 1, 1, _Ticker(_sel(toks, tp1), n1))
            for u in range(pb):
                qkv_part(1, u)
                if u == 0:
                    attn(0, ng - 1)
                else:
                    attn(1, u - 1)
        with scope("w_2"):
            cp_wo.wait()
            cp_modb.wait()
            cp_x(2).wait()
        cp_x(3).start()
        cp_x(4).start()
        for cp in [cp_x(i) for i in range(5, NA)] + [cp_modc]:
            cp.start(priority=xp)
        for j in range(nf):
            for k in range(3):
                cp_f(k, j).start(priority=1)
        with scope("a_1"):
            pieces = []
            cuts = [2 * D + int(v) * L for v in str(mcut).split('x')] + [2944]
            hooks = [(lambda lo=lo, hi=hi: pieces.append(mod_cols(lo, hi))) for lo, hi in zip(cuts, cuts[1:])]
            hooks.pop(0)()
            toks = []
            for u in range(pb, ng):
                toks += qkv_part(1, u, hooks)
                attn(1, u - 1)
            while hooks:
                hooks.pop(0)()
            mod = jnp.concatenate(pieces, axis=1)
            woT[...] = pltpu.bitcast((wo_v[...].astype(f32) * mod[0:1, 0:D]).astype(bf16).T, u32)
            modr[0] = mod[:, D:2 * D]
            modr[1] = mod[:, 2 * D:3 * D] + 1.0
            toks += wo_res(0)
            attn(1, ng - 1)
            ln1(2, 2, 0, _Ticker(toks[len(toks) // 4:-16], n1))

        cp_x(3).wait()
        cp_x(4).wait()

        def a_tile(i, last=False):
            toks = []
            for u in range(ng):
                toks += qkv_part(i, u)
                if u > 0:
                    attn(i, u - 1)
            h2 = ln2a(i - 2, _Ticker(_sel(toks, t2a), n2a))
            toks += wo_res(i - 1)
            attn(i, ng - 1)
            ln2b(i - 2, h2, _Ticker(_sel(toks, t2b), n2b))
            if not last:
                ln1(jnp.minimum(_iv(i) + 1, NA - 1), jnp.minimum(_iv(i), NA - 2) + 1, (i + 1) % 2, _Ticker(_sel(toks, t1), n1))

        def a_body(it, carry):
            i0 = 2 + it * aun
            with scope("w_x"):
                @pl.when(it == 1)
                def _():
                    for i in range(5, NA):
                        cp_x(i).wait()
                    cp_modc.wait()
            with scope("a_body"):
                for d in range(aun):
                    a_tile(_Idx(i0, d) if aun % 2 == 0 else i0 + d)
            return carry

        jax.lax.fori_loop(0, (NA - 2 - apl) // aun, a_body, 0)
        for buf in (w1_v, w3_v, w2t_v):
            pltpu.make_async_copy(buf, buf, sem.at[2]).wait()
        with scope("a_epi"):
            for i in range(NA - apl, NA):
                a_tile(i, i == NA - 1)
            modb[2] = col_bcast(mod_cols(2816, 6 * D)[:, 5 * D - 2816:])
            toks = wo_res(NA - 1)
            ln2(NA - 2, notick, _Ticker(_sel(toks, te), n2b))
            ln2(NA - 1, notick, notick)

        def cp_o(ii, ri):
            rows = pl.ds(ri * QD, QD)
            return pltpu.make_async_copy(out_v.at[ii, rows], out_hbm.at[rows, pl.ds(ii * 2 * TA, 2 * TA)],
                                         sem.at[3])

        QS = ((0, 0), (0, 1), (1, 0), (1, 1))

        def strassen_out(get, init=None):
            cacc = dict(init) if init else {}
            for a in range(7):
                p = [get(a, b) for b in range(7)]
                inn = {(0, 0): p[0] + p[3] - p[4] + p[6], (0, 1): p[2] + p[4],
                       (1, 0): p[1] + p[3], (1, 1): p[0] - p[1] + p[2] + p[5]}
                for tgt, sign in SOUT[a]:
                    for q in QS:
                        key = tgt + q
                        if key not in cacc:
                            cacc[key] = inn[q]
                        else:
                            cacc[key] = cacc[key] + inn[q] if sign > 0 else cacc[key] - inn[q]
            return cacc

        def fin(ii, ri, tk):
            cs = slice(ii * L, (ii + 1) * L)
            lo = jax.lax.broadcasted_iota(jnp.int32, (fr, L), 1) < 64
            for r in range(0, QD, fr):
                tick = tk()
                if tick is not None:
                    tick = jnp.concatenate([tick] * (fr // 8), axis=0)
                cc = _hk_c_row(lambda k: acc[k, r:r + fr, cs], ri, tick)
                rows = slice(ri * QD + r, ri * QD + r + fr)
                res = [[], []]
                for a1 in range(2):
                    v0, v1 = cc[2 * a1], cc[2 * a1 + 1]
                    z = pltpu.roll(jnp.where(lo, v1, v0), 64, 1)
                    for par, v in enumerate((jnp.where(lo, v0, z), jnp.where(lo, z, v1))):
                        res[par].append(x1_sc[2 * (2 * ii + par) + a1, rows] + modb[2, rows] * v)
                out_v[ii, rows, :] = jnp.concatenate(res[0] + res[1], axis=1).astype(bf16)

        n_early = units[-1][0] // L

        def b_body(j, carry):
            if skipb:
                acc[0, 0:64, 0:L] += _upk(a_sc[j, 0:32, :]).astype(f32) + _upk(t_sc[0, 0:32, :]).astype(f32)[:, 0:1]
                return carry
            bw = {}
            for c1, wv in enumerate((w1_v, w3_v)):
                lv1 = _sb(wv[j, 0:256, 0:hf].astype(f32), wv[j, 0:256, hf:tf].astype(f32),
                          wv[j, 256:512, 0:hf].astype(f32), wv[j, 256:512, hf:tf].astype(f32))
                for a in OORD:
                    y = lv1[a]
                    for b, v in enumerate(_sb(y[0:L, 0:L], y[0:L, L:], y[L:, 0:L], y[L:, L:])):
                        bw[(a, b, c1)] = v.astype(bf16)
            aw = [v.astype(bf16) for v in _hk_a(
                [w2t_v[j, i * QD:(i + 1) * QD, 0:hf].astype(f32) for i in range(4)],
                [w2t_v[j, i * QD:(i + 1) * QD, hf:tf].astype(f32) for i in range(4)])]

            def gu(tt):
                st, sz = units[tt]
                rq = slice(st // 4, (st + sz) // 4)
                prods = {}

                def main(c1):
                    for a in OORD:
                        for b in OORD:
                            prods[(c1, a, b)] = jnp.dot(_upk(a_sc[7 * a + b, rq, :]), bw[(a, b, c1)],
                                                        preferred_element_type=f32)

                def tail(c1, a1, a2, c2, nn):
                    wv = (w1_v, w3_v)[c1]
                    col = c2 * hf + nn * L
                    prods[(c1, 't', a1, a2, c2, nn)] = jnp.dot(
                        _upk(t_sc[2 * a1 + a2, rq, :]), wv[j, 512:576, col:col + L],
                        preferred_element_type=f32)

                if gord == 0:
                    for c1 in range(2):
                        main(c1)
                        for a1, a2 in QS:
                            for c2, nn in QS:
                                tail(c1, a1, a2, c2, nn)
                else:
                    main(0)
                    main(1)
                    for a1, a2 in QS:
                        for c2, nn in QS:
                            for c1 in range(2):
                                tail(c1, a1, a2, c2, nn)
                return prods

            def combine(prods):
                nf_ = (lambda v: jnp.concatenate([v[0:64], v[64:]], axis=0)) if nofuse else (lambda v: v)
                gu_ = []
                for c1 in range(2):
                    init = {(a1, c2, a2, nn): nf_(prods[(c1, 't', a1, a2, c2, nn)])
                            for a1, c2 in QS for a2, nn in QS}
                    gu_.append(strassen_out(lambda a, b: nf_(prods[(c1, a, b)]), init))
                e = {(a1, a2, c2, nn): _silu_mul(gu_[0][(a1, c2, a2, nn)], gu_[1][(a1, c2, a2, nn)])
                     for a1, a2 in QS for c2, nn in QS}
                blk = lambda a1, a2, c2: jnp.concatenate([e[(a1, a2, c2, nn)] for nn in range(2)], axis=1)
                return [v.astype(bf16) for v in _hk_b([blk(a1, a2, 0) for a1, a2 in QS],
                                                      [blk(a1, a2, 1) for a1, a2 in QS])]

            def down(tt, eb):
                st, sz = units[tt]
                rs = slice(st // 2, (st + sz) // 2)
                toks = []
                for k in DORD:
                    d = jax.lax.dot_general(aw[k], eb[k], NT, preferred_element_type=f32)
                    acc[k, :, rs] += d
                    toks.append(d)
                return toks

            def finish(tt, toks):
                pairs = range(units[tt][0] // (2 * L), (units[tt][0] + units[tt][1]) // (2 * L))
                toks = [v[r:r + 8, 0:L] for v in toks[::fst] for r in range(0, v.shape[0], 16)]
                tk = _Ticker(toks if fpace else None, 4 * len(pairs) * (QD // fr))
                for ii in pairs:
                    for ri in range(4):
                        fin(ii, ri, tk)

                        @pl.when(j == nf - 1)
                        def _():
                            cp_o(ii, ri).start()

            def gtoks(prods):
                return [v for k, v in prods.items() if k[1] != 't']

            eb = combine(gu(0))
            for tt in range(nsup):
                prn = gu(tt + 1) if tt + 1 < nsup else None
                ebn = combine(prn) if prn is not None else None
                if tt > 0 and prn is not None and dofin:
                    finish(tt - 1, gtoks(prn)[ga:gb_])
                dt = down(tt, eb)
                if tt > 0 and prn is None and dofin:
                    finish(tt - 1, dt[da:db])
                eb = ebn
            return carry

        with scope("b_loop"):
            jax.lax.fori_loop(0, nf, b_body, 0)

        with scope("fin"):
            for ii in range(n_early // 2, NA // 2):
                for ri in range(4):
                    fin(ii, ri, notick)
                    cp_o(ii, ri).start()
        with scope("w_out"):
            pltpu.make_async_copy(out_v, out_v, sem.at[3]).wait()

    def fn(A_x, A_wqkv, A_wo, B_x, B_w1, B_w3, B_w2, c, w_mod):
        xT = A_x.reshape(S, D).T
        w2t = B_w2.T
        hbm = pl.BlockSpec(memory_space=pl.ANY)
        outT = pl.pallas_call(
            kernel,
            in_specs=[hbm] * 8,
            out_specs=hbm,
            out_shape=jax.ShapeDtypeStruct((D, S), bf16),
            scratch_shapes=[
                pltpu.VMEM((1, D), bf16),
                pltpu.VMEM((NA, D, TA), bf16),
                pltpu.VMEM((D, 6 * D), bf16),
                pltpu.VMEM((D, 3 * D), bf16),
                pltpu.VMEM((3 * D // 2, D), u32),
                pltpu.VMEM((D, D), bf16),
                pltpu.VMEM((D // 2, D), u32),
                pltpu.VMEM((nf, D, tf), bf16),
                pltpu.VMEM((nf, D, tf), bf16),
                pltpu.VMEM((nf, D, tf), bf16),
                pltpu.VMEM((3, D, L), f32),
                pltpu.VMEM((2, 8, D), f32),
                pltpu.VMEM((2, 2, D, L), f32),
                pltpu.VMEM((2, H // hg, hg * DH, L), f32),
                pltpu.VMEM((2 * NA + 1, H // hg, hg * DH, L), u32),
                pltpu.VMEM((2, 2, D, L), f32),
                pltpu.VMEM((2 * NA, D, L), f32),
                pltpu.VMEM((2 * NA, 3, 8, L), f32),
                pltpu.VMEM((49, S // 8, L), u32),
                pltpu.VMEM((4, S // 8, 64), u32),
                pltpu.VMEM((26, D // 4, S // 4), f32),
                pltpu.VMEM((NA // 2, D, 2 * TA), bf16),
                pltpu.SemaphoreType.DMA((6,)),
            ],
            compiler_params=pltpu.CompilerParams(vmem_limit_bytes=100 * 1024 * 1024),
        )(xT, c, w_mod, A_wqkv, A_wo, B_w1, B_w3, w2t)
        return outT.T.reshape(1, S, D)

    return fn


pallas_adaLN_cond__sliding_local_dilated__glu_gated_swiglu__prompt_kernel = jax.jit(make())
```

```python
import jax
import jax.numpy as jnp
import jax.experimental.pallas as pl
import jax.experimental.pallas.tpu as pltpu

S, D, F, H, DH, W, DIL = 2048, 576, 4608, 32, 18, 8, 2
f32 = jnp.float32
bf16 = jnp.bfloat16
u32 = jnp.uint32
NT = (((1,), (1,)), ((), ()))

L = 128
TA = 256
NA = S // TA
HG = 8
NG = H // HG
HR = HG * DH
GR = 3 * HR
QD = D // 4
TF = 512
HF = TF // 2
NF = F // TF
UNITS = ((0, 4), (4, 2), (6, 2))
QS = ((0, 0), (0, 1), (1, 0), (1, 1))

WQ = ((0, 384), (512, 896), (1152, 1536), (384, 512), (896, 1152), (1536, 1728))
MOD_A, MOD_B = 2 * D, 2944

SORD = (4, 1, 0, 3, 2, 6, 5)
SIN = (((0, 0), (1, 1), 1), ((1, 0), (1, 1), 1), ((0, 0), None, 0), ((1, 1), None, 0),
       ((0, 0), (0, 1), 1), ((1, 0), (0, 0), -1), ((0, 1), (1, 1), -1))
SOUT = ((((0, 0), 1), ((1, 1), 1)), (((1, 0), 1), ((1, 1), -1)), (((0, 1), 1), ((1, 1), 1)),
        (((0, 0), 1), ((1, 0), 1)), (((0, 0), -1), ((0, 1), 1)), (((1, 1), 1),), (((0, 0), 1),))

LAM = (-2.0, -0.5, 0.5, 2.0)
PAIRS = tuple((i, j) for i in range(4) for j in range(i + 1, 4))
DORD = (4, 0, 5, 1, 8, 9, 10, 6, 2, 11, 12, 13, 17, 18, 19, 7, 3, 14, 15, 16, 20, 21, 22, 23, 24, 25)

C2 = 48
N_LN1 = 2 * (D // 16)
N_LN2A = 2 * (D // C2)
N_LN2B = 7 * 4


class _Ticker:
    def __init__(self, toks=None, n=1):
        self.toks, self.n, self.k = toks, n, 0

    def __call__(self):
        if not self.toks:
            return None
        tok = self.toks[min(self.k * len(self.toks) // self.n, len(self.toks) - 1)]
        self.k += 1
        return jnp.where(tok > jnp.inf, 1.0, 0.0)


class _Idx:
    def __init__(self, base, off=0):
        self.base, self.off = base, off

    def __add__(self, k):
        return _Idx(self.base, self.off + k)

    def __sub__(self, k):
        return _Idx(self.base, self.off - k)

    def __mod__(self, m):
        assert m == 2
        return self.off % 2

    def __rmul__(self, k):
        return k * self.base + k * self.off

    __mul__ = __rmul__


def _iv(i):
    return i.base + i.off if isinstance(i, _Idx) else i


def _toks(res):
    return [res[r:r + 8, t * L:(t + 1) * L]
            for t in range(res.shape[1] // L) for r in range(0, res.shape[0], 8)]


def _plus(v, tick):
    if tick is None:
        return v
    n = v.shape[1] // L
    return v + (tick if n == 1 else jnp.concatenate([tick] * n, axis=1))


def _stats(k8, s1, s2):
    md = jnp.sum(s1, axis=0, keepdims=True) * (1.0 / D)
    var = jnp.sum(s2, axis=0, keepdims=True) * (1.0 / D) - md * md
    rs = jax.lax.rsqrt(jnp.maximum(var, 0.0) + 1e-5)
    return k8 + md, jnp.broadcast_to(rs, k8.shape)


def _silu_mul(g, u):
    hg = 0.5 * g
    return (hg * jnp.tanh(hg) + hg) * u


def _sa(x11, x12, x21, x22):
    return [x11 + x22, x21 + x22, x11, x22, x11 + x12, x21 - x11, x12 - x22]


def _sb(y11, y12, y21, y22):
    return [y11 + y22, y11, y12 - y22, y21 - y11, y22, y11 + y12, y21 + y22]


def _strassen_out(get, cacc):
    cacc = dict(cacc)
    for a in range(7):
        p = [get(a, b) for b in range(7)]
        inn = {(0, 0): p[0] + p[3] - p[4] + p[6], (0, 1): p[2] + p[4],
               (1, 0): p[1] + p[3], (1, 1): p[0] - p[1] + p[2] + p[5]}
        for tgt, sign in SOUT[a]:
            for q in QS:
                cacc[tgt + q] = cacc[tgt + q] + inn[q] if sign > 0 else cacc[tgt + q] - inn[q]
    return cacc


def _hk_a(x, y):
    z = [[y[i] + LAM[l] * x[i] for i in range(4)] for l in range(4)]
    ops = [x[i] for i in range(4)] + [z[i][i] for i in range(4)]
    for i, j in PAIRS:
        r = 1.0 / (LAM[i] - LAM[j])
        ops += [(z[i][i] - z[j][j]) * r, (z[j][i] - z[j][j]) * r, (z[i][j] - z[i][i]) * r]
    return ops


def _hk_b(b1, b2):
    u = [b1[i] - LAM[i] * b2[i] for i in range(4)]
    ops = u + list(b2)
    for i, j in PAIRS:
        ops += [u[i] + u[j], (u[i] + b1[j]) - LAM[i] * b2[j], (u[j] + b1[i]) - LAM[j] * b2[i]]
    return ops


def _hk_c_row(m, i, tick):
    p = _plus(m(i), tick)
    out = []
    for j in range(4):
        if j == i:
            out.append(p + m(4 + i))
        else:
            k = 8 + 3 * PAIRS.index((min(i, j), max(i, j)))
            v = (m(4 + j) - p) + m(k)
            out.append(v - m(k + 1) if i < j else v + m(k + 2))
    return out


def _pk(v):
    return pltpu.bitcast(v.astype(bf16), u32)


def _upk(v):
    return pltpu.bitcast(v, bf16)


def _kernel(x_hbm, c_hbm, wmod_hbm, wqkv_hbm, wo_hbm, w1_hbm, w3_hbm, w2t_hbm, out_hbm,
            c_v, x_v, wmod_v, wqkv_v, wqkvT, wo_v, woT, w1_v, w3_v, w2t_v,
            modb, modr, h_sc, q_sc, k_sc, v_sc, o_sc, x1_sc, st_sc, a_sc, t_sc, acc, out_v,
            sem):
    def cp_x(i):
        s = {1: 4, 2: 5}.get(i, 0)
        return pltpu.make_async_copy(x_hbm.at[:, pl.ds(i * TA, TA)], x_v.at[i], sem.at[s])

    def cp_f(k, j):
        src, dst = ((w1_hbm, w1_v), (w3_hbm, w3_v), (w2t_hbm, w2t_v))[k]
        return pltpu.make_async_copy(src.at[:, pl.ds(j * TF, TF)], dst.at[j], sem.at[2])

    def cp_cols(src, dst, lo, hi, s):
        return pltpu.make_async_copy(src.at[:, pl.ds(lo, hi - lo)], dst.at[:, pl.ds(lo, hi - lo)], sem.at[s])

    def cp_wq(k):
        return cp_cols(wqkv_hbm, wqkv_v, WQ[k][0], WQ[k][1], min(1 + k, 4))

    def cp_o(ii, ri):
        rows = pl.ds(ri * QD, QD)
        return pltpu.make_async_copy(out_v.at[ii, rows], out_hbm.at[rows, pl.ds(ii * 2 * TA, 2 * TA)],
                                     sem.at[3])

    cp_moda = cp_cols(wmod_hbm, wmod_v, 0, MOD_A, 0)
    cp_modb = cp_cols(wmod_hbm, wmod_v, MOD_A, MOD_B, 5)
    cp_modc = cp_cols(wmod_hbm, wmod_v, MOD_B, 6 * D, 2)
    cp_c = pltpu.make_async_copy(c_hbm, c_v, sem.at[0])
    cp_wo = pltpu.make_async_copy(wo_hbm, wo_v, sem.at[5])

    cp_moda.start()
    cp_x(0).start()
    cp_c.start()
    for cp in [cp_wq(k) for k in range(6)] + [cp_x(1), cp_wo, cp_modb, cp_x(2)]:
        cp.start(priority=1)

    acc[...] = jnp.zeros(acc.shape, f32)
    k_sc[0] = jnp.zeros(k_sc.shape[1:], u32)
    v_sc[0] = jnp.zeros(v_sc.shape[1:], f32)

    def mod_cols(lo, hi):
        c = c_v[...].astype(f32)
        sc = jnp.broadcast_to((c * jax.nn.sigmoid(c)).astype(bf16), (16, D))
        return jnp.dot(sc, wmod_v[:, lo:hi], preferred_element_type=f32)[0:8]

    def col_bcast(row):
        return jnp.broadcast_to(row[0:1], (L, D)).T

    def tr_wq(k):
        lo, hi = WQ[k]
        wt = pltpu.bitcast(wqkv_v[:, lo:hi].T, u32)
        c = lo
        while c < hi:
            e = min(hi, (c // HR + 1) * HR)
            dst = (c % D) // HR * GR + c // D * HR + c % HR
            wqkvT[dst // 2:(dst + e - c) // 2, :] = wt[(c - lo) // 2:(e - lo) // 2, :]
            c = e

    def ln1(i, i2, slot, tk):
        k8 = jnp.broadcast_to(x_v[i, 0:16, :].astype(f32)[0:1], (8, TA))
        s1 = s2 = None
        for r in range(0, D, 16):
            kk = _plus(k8, tk())
            x = x_v[i, r:r + 16, :].astype(f32)
            for h in range(2):
                d = x[8 * h:8 * h + 8] - kk
                s1 = d if s1 is None else s1 + d
                s2 = d * d if s2 is None else s2 + d * d
        m8, rs8 = _stats(k8, s1, s2)
        for r in range(0, D, 16):
            mk = _plus(m8, tk())
            x = x_v[i2, r:r + 16, :].astype(f32)
            rows = []
            for h in range(2):
                rr = slice(r + 8 * h, r + 8 * h + 8)
                xn = (x[8 * h:8 * h + 8] - mk) * rs8
                rows.append(jnp.concatenate(
                    [xn[:, t * L:(t + 1) * L] * modb[1, rr] + modb[0, rr] for t in range(2)], axis=1))
            h_sc[slot, r // 2:r // 2 + 8] = _pk(jnp.concatenate(rows, axis=0))

    def qkv_part(i, u, hooks=None):
        h = _upk(h_sc[i % 2])
        toks, res = [], []
        for r in range(3):
            lo = (u * GR + r * HR) // 2
            res.append(jnp.dot(_upk(wqkvT[lo:lo + HR // 2, :]), h, preferred_element_type=f32))
            toks += _toks(res[r])
            if hooks:
                hooks.pop(0)()
        for t in range(2):
            q_sc[t, u] = res[0][:, t * L:(t + 1) * L]
            k_sc[2 * i + t + 1, u] = _pk(res[1][:, t * L:(t + 1) * L])
            v_sc[2 * i + t + 1, u] = res[2][:, t * L:(t + 1) * L]
        return toks

    def attn(i, u):
        lane = jax.lax.broadcasted_iota(jnp.int32, (HG, L), 1)

        def shift(cur, prev, w):
            return pltpu.roll(jnp.where(lane < L - DIL * w, cur, prev), DIL * w, 1)

        def weights(t):
            g = 2 * i + t
            lg = [None] * W
            for p in range(DH // 2):
                q0 = q_sc[t, u, pl.ds(2 * p, HG, stride=DH), :]
                q1 = q_sc[t, u, pl.ds(2 * p + 1, HG, stride=DH), :]
                cur = k_sc[g + 1, u, pl.ds(p, HG, stride=DH // 2), :]
                prev = k_sc[g, u, pl.ds(p, HG, stride=DH // 2), :]
                for w in range(W):
                    kw = cur if w == 0 else shift(cur, prev, w)
                    k0 = pltpu.bitcast(kw << 16, f32)
                    k1 = pltpu.bitcast(kw & jnp.uint32(0xFFFF0000), f32)
                    tmp = q0 * k0 + q1 * k1
                    lg[w] = tmp if lg[w] is None else lg[w] + tmp
            pos = lane + g * L
            lg = [v * (DH ** -0.5) for v in lg]
            for w in range(1, W):
                lg[w] = jnp.where(pos >= DIL * w, lg[w], -1e9)
            m = lg[0]
            for w in range(1, W):
                m = jnp.maximum(m, lg[w])
            es = [jnp.exp(v - m) for v in lg]
            den = es[0]
            for w in range(1, W):
                den = den + es[w]
            inv = 1.0 / den
            return [e * inv for e in es]

        def values(t, at):
            g = 2 * i + t
            for d in range(DH):
                cur = v_sc[g + 1, u, pl.ds(d, HG, stride=DH), :]
                prev = v_sc[g, u, pl.ds(d, HG, stride=DH), :]
                o = at[0] * cur
                for w in range(1, W):
                    o = o + at[w] * shift(cur, prev, w)
                o_sc[i % 2, t, pl.ds(u * HR + d, HG, stride=DH), :] = o

        ats = [weights(t) for t in range(2)]
        for t in range(2):
            values(t, ats[t])

    def wo_res(i):
        o = jnp.concatenate([o_sc[i % 2, 0], o_sc[i % 2, 1]], axis=1).astype(bf16)
        mo = D // 2
        k8, s1, s2 = [None] * 2, [None] * 2, [None] * 2
        toks = []
        for r in range(2):
            att = jnp.dot(_upk(woT[r * mo // 2:(r + 1) * mo // 2, :]), o, preferred_element_type=f32)
            toks += _toks(att)
            rs = slice(r * mo, (r + 1) * mo)
            x = x_v[_iv(i), rs, :].astype(f32)
            for t in range(2):
                x1 = x[:, t * L:(t + 1) * L] + att[:, t * L:(t + 1) * L]
                x1_sc[2 * i + t, rs] = x1
                if r == 0:
                    k8[t] = jnp.broadcast_to(x1[0:1], (8, L))
                for q in range(0, mo, 8):
                    d = x1[q:q + 8] - k8[t]
                    s1[t] = d if s1[t] is None else s1[t] + d
                    s2[t] = d * d if s2[t] is None else s2[t] + d * d
        for t in range(2):
            st_sc[2 * i + t, 0], st_sc[2 * i + t, 1], st_sc[2 * i + t, 2] = k8[t], s1[t], s2[t]
        return toks

    def ln2a(i, tk):
        h2 = []
        for t in range(2):
            m8, rs8 = _stats(st_sc[2 * i + t, 0], st_sc[2 * i + t, 1], st_sc[2 * i + t, 2])
            rows = []
            for r in range(0, D, 8):
                if r % C2 == 0:
                    mk = _plus(m8, tk())
                rows.append((x1_sc[2 * i + t, r:r + 8] - mk) * rs8)
            h2.append(jnp.concatenate(rows, axis=0).T * modr[1, 0:1] + modr[0, 0:1])
        return h2

    def ln2b(i, h2, tk):
        r0 = i * 32 if isinstance(i, int) else pl.multiple_of(i * 32, 32)
        for a1, a2 in QS:
            t_sc[2 * a1 + a2, pl.ds(r0, 32), :] = _pk(h2[a1][64 * a2:64 * a2 + 64, 512:D])
        blk = ((h2[0][:, 0:256], h2[0][:, 256:512]), (h2[1][:, 0:256], h2[1][:, 256:512]))
        for a in (2, 4, 5, 0, 1, 3, 6):
            p0, p1, sgn = SIN[a]
            for r in range(0, 64, 16):
                tick = tk()
                xs = []
                for a2 in range(2):
                    rows = []
                    for q in range(64 * a2 + r, 64 * a2 + r + 16, 8):
                        v = _plus(blk[p0[0]][p0[1]][q:q + 8], tick)
                        if p1 is not None:
                            o = blk[p1[0]][p1[1]][q:q + 8]
                            v = v + o if sgn > 0 else v - o
                        rows.append(v)
                    xs.append(jnp.concatenate(rows, axis=0))
                for b, v in enumerate(_sa(xs[0][:, 0:L], xs[0][:, L:], xs[1][:, 0:L], xs[1][:, L:])):
                    a_sc[7 * a + b, pl.ds(r0 + r // 2, 8), :] = _pk(v)

    notick = _Ticker()
    cp_c.wait()
    cp_moda.wait()
    cp_x(0).wait()
    mod = mod_cols(0, MOD_A)
    modb[0] = col_bcast(mod[:, 0:D])
    modb[1] = col_bcast(mod[:, D:2 * D] + 1.0)
    ln1(0, 0, 0, notick)

    for k in range(3):
        cp_wq(k).wait()
        tr_wq(k)
    qkv_part(0, 0)
    qkv_part(0, 1)
    attn(0, 0)

    for k in range(3, 6):
        cp_wq(k).wait()
    cp_x(1).wait()
    for k in range(3, 6):
        tr_wq(k)
    toks = []
    for u in range(2, NG):
        toks += qkv_part(0, u)
        attn(0, u - 1)
    ln1(1, 1, 1, _Ticker(toks[0:150], N_LN1))
    for u in range(NG - 1):
        qkv_part(1, u)
        if u == 0:
            attn(0, NG - 1)
        else:
            attn(1, u - 1)

    cp_wo.wait()
    cp_modb.wait()
    cp_x(2).wait()
    for i in range(3, NA):
        cp_x(i).start()
    cp_modc.start(priority=1)
    for j in range(NF):
        for k in range(3):
            cp_f(k, j).start(priority=1)
    pieces = []
    cuts = [MOD_A + v * L for v in (0, 5, 8, 11)] + [MOD_B]
    hooks = [(lambda lo=lo, hi=hi: pieces.append(mod_cols(lo, hi))) for lo, hi in zip(cuts, cuts[1:])]
    hooks.pop(0)()
    toks = qkv_part(1, NG - 1, hooks)
    attn(1, NG - 2)
    mod = jnp.concatenate(pieces, axis=1)
    woT[...] = pltpu.bitcast((wo_v[...].astype(f32) * mod[0:1, 0:D]).astype(bf16).T, u32)
    modr[0] = mod[:, D:2 * D]
    modr[1] = mod[:, 2 * D:3 * D] + 1.0
    toks += wo_res(0)
    attn(1, NG - 1)
    ln1(2, 2, 0, _Ticker(toks[len(toks) // 4:-16], N_LN1))

    for i in range(3, NA):
        cp_x(i).wait()

    def a_tile(i):
        toks = []
        for u in range(NG):
            toks += qkv_part(i, u)
            if u > 0:
                attn(i, u - 1)
        h2 = ln2a(i - 2, notick)
        toks += wo_res(i - 1)
        attn(i, NG - 1)
        ln2b(i - 2, h2, _Ticker(toks[20:108] + toks[490:570], N_LN2B))
        ln1(jnp.minimum(_iv(i) + 1, NA - 1), jnp.minimum(_iv(i), NA - 2) + 1, (i + 1) % 2,
            _Ticker(toks[108:500], N_LN1))

    def a_body(it, carry):
        for d in range(2):
            a_tile(_Idx(2 + 2 * it, d))
        return carry

    jax.lax.fori_loop(0, (NA - 2) // 2, a_body, 0)

    cp_modc.wait()
    for j in range(NF):
        for k in range(3):
            cp_f(k, j).wait()
    modb[2] = col_bcast(mod_cols(MOD_B - L, 6 * D)[:, 5 * D - (MOD_B - L):])
    toks = wo_res(NA - 1)
    ln2b(NA - 2, ln2a(NA - 2, notick), _Ticker(toks[0:100], N_LN2B))

    def fin(ii, ri, tk):
        cs = slice(ii * L, (ii + 1) * L)
        lo = jax.lax.broadcasted_iota(jnp.int32, (8, L), 1) < 64
        for r in range(0, QD, 8):
            cc = _hk_c_row(lambda k: acc[k, r:r + 8, cs], ri, tk())
            rows = slice(ri * QD + r, ri * QD + r + 8)
            res = [[], []]
            for a1 in range(2):
                v0, v1 = cc[2 * a1], cc[2 * a1 + 1]
                z = pltpu.roll(jnp.where(lo, v1, v0), 64, 1)
                for par, v in enumerate((jnp.where(lo, v0, z), jnp.where(lo, z, v1))):
                    res[par].append(x1_sc[2 * (2 * ii + par) + a1, rows] + modb[2, rows] * v)
            out_v[ii, rows, :] = jnp.concatenate(res[0] + res[1], axis=1).astype(bf16)

    def b_body(j, carry):
        bw = {}
        for c1, wv in enumerate((w1_v, w3_v)):
            lv1 = _sb(wv[j, 0:256, 0:HF].astype(f32), wv[j, 0:256, HF:TF].astype(f32),
                      wv[j, 256:512, 0:HF].astype(f32), wv[j, 256:512, HF:TF].astype(f32))
            for a in SORD:
                y = lv1[a]
                for b, v in enumerate(_sb(y[0:L, 0:L], y[0:L, L:], y[L:, 0:L], y[L:, L:])):
                    bw[(c1, a, b)] = v.astype(bf16)
        aw = [v.astype(bf16) for v in _hk_a(
            [w2t_v[j, i * QD:(i + 1) * QD, 0:HF].astype(f32) for i in range(4)],
            [w2t_v[j, i * QD:(i + 1) * QD, HF:TF].astype(f32) for i in range(4)])]

        def gate_up(tt):
            t0, nt = UNITS[tt]
            rq = slice(t0 * 32, (t0 + nt) * 32)
            main, rem = {}, {}
            for c1 in range(2):
                for a in SORD:
                    for b in SORD:
                        main[(c1, a, b)] = jnp.dot(_upk(a_sc[7 * a + b, rq, :]), bw[(c1, a, b)],
                                                   preferred_element_type=f32)
            for a1, a2 in QS:
                for c2, nn in QS:
                    for c1, wv in enumerate((w1_v, w3_v)):
                        col = c2 * HF + nn * L
                        rem[(c1, a1, c2, a2, nn)] = jnp.dot(
                            _upk(t_sc[2 * a1 + a2, rq, :]), wv[j, 512:D, col:col + L],
                            preferred_element_type=f32)
            keep = lambda v: jnp.concatenate([v[0:64], v[64:]], axis=0)
            g, u = [_strassen_out(lambda a, b: keep(main[(c1, a, b)]),
                                  {k1 + k2: keep(rem[(c1,) + k1 + k2]) for k1 in QS for k2 in QS})
                    for c1 in range(2)]
            act = {k: _silu_mul(g[k], u[k]) for k in g}
            blk = lambda a1, a2, c2: jnp.concatenate([act[(a1, c2, a2, nn)] for nn in range(2)], axis=1)
            eb = [v.astype(bf16) for v in _hk_b([blk(a1, a2, 0) for a1, a2 in QS],
                                                [blk(a1, a2, 1) for a1, a2 in QS])]
            return eb, list(main.values())

        def down(tt, eb):
            t0, nt = UNITS[tt]
            res = []
            for k in DORD:
                d = jax.lax.dot_general(aw[k], eb[k], NT, preferred_element_type=f32)
                acc[k, :, t0 * 64:(t0 + nt) * 64] += d
                res.append(d)
            return res

        def finish(tt, prods):
            t0, nt = UNITS[tt]
            toks = [v[r:r + 8, 0:L] for v in prods for r in range(0, v.shape[0], 16)]
            tk = _Ticker(toks, 2 * nt * (QD // 8))
            for ii in range(t0 // 2, (t0 + nt) // 2):
                for ri in range(4):
                    fin(ii, ri, tk)

                    @pl.when(j == NF - 1)
                    def _():
                        cp_o(ii, ri).start()

        eb0, _ = gate_up(0)
        eb1, prods = gate_up(1)
        gt = [v[r:r + 8] for v in prods for r in range(0, v.shape[0], 32)]
        n = len(gt)
        ln2b(NA - 1, ln2a(NA - 1, _Ticker(gt[n * 5 // 100:n * 30 // 100], N_LN2A)),
             _Ticker(gt[n * 35 // 100:n * 95 // 100], N_LN2B))
        down(0, eb0)
        eb2, prods = gate_up(2)
        finish(0, prods[4:88])
        down(1, eb1)
        finish(1, down(2, eb2)[2:22])
        return carry

    jax.lax.fori_loop(0, NF, b_body, 0)

    for ri in range(4):
        fin(NA // 2 - 1, ri, notick)
        cp_o(NA // 2 - 1, ri).start()
    for ii in range(NA // 2):
        for ri in range(4):
            cp_o(ii, ri).wait()


@jax.jit
def pallas_adaLN_cond__sliding_local_dilated__glu_gated_swiglu__prompt_kernel(
    A_x: jax.Array,
    A_wqkv: jax.Array,
    A_wo: jax.Array,
    B_x: jax.Array,
    B_w1: jax.Array,
    B_w3: jax.Array,
    B_w2: jax.Array,
    c: jax.Array,
    w_mod: jax.Array,
):
    del B_x
    hbm = pl.BlockSpec(memory_space=pl.ANY)
    out_t = pl.pallas_call(
        _kernel,
        in_specs=[hbm] * 8,
        out_specs=hbm,
        out_shape=jax.ShapeDtypeStruct((D, S), bf16),
        scratch_shapes=[
            pltpu.VMEM((1, D), bf16),
            pltpu.VMEM((NA, D, TA), bf16),
            pltpu.VMEM((D, 6 * D), bf16),
            pltpu.VMEM((D, 3 * D), bf16),
            pltpu.VMEM((3 * D // 2, D), u32),
            pltpu.VMEM((D, D), bf16),
            pltpu.VMEM((D // 2, D), u32),
            pltpu.VMEM((NF, D, TF), bf16),
            pltpu.VMEM((NF, D, TF), bf16),
            pltpu.VMEM((NF, D, TF), bf16),
            pltpu.VMEM((3, D, L), f32),
            pltpu.VMEM((2, 8, D), f32),
            pltpu.VMEM((2, D // 2, TA), u32),
            pltpu.VMEM((2, NG, HR, L), f32),
            pltpu.VMEM((2 * NA + 1, NG, HR // 2, L), u32),
            pltpu.VMEM((2 * NA + 1, NG, HR, L), f32),
            pltpu.VMEM((2, 2, D, L), f32),
            pltpu.VMEM((2 * NA, D, L), f32),
            pltpu.VMEM((2 * NA, 3, 8, L), f32),
            pltpu.VMEM((49, S // 8, L), u32),
            pltpu.VMEM((4, S // 8, 64), u32),
            pltpu.VMEM((26, QD, S // 4), f32),
            pltpu.VMEM((NA // 2, D, 2 * TA), bf16),
            pltpu.SemaphoreType.DMA((6,)),
        ],
        compiler_params=pltpu.CompilerParams(vmem_limit_bytes=100 * 1024 * 1024),
    )(A_x.reshape(S, D).T, c, w_mod, A_wqkv, A_wo, B_w1, B_w3, B_w2.T)
    return out_t.T.reshape(1, S, D)
```

```python
import jax
import jax.numpy as jnp
import jax.experimental.pallas as pl
import jax.experimental.pallas.tpu as pltpu

S, D, F, H, DH, W, DIL = 2048, 576, 4608, 32, 18, 8, 2
f32 = jnp.float32
bf16 = jnp.bfloat16
u32 = jnp.uint32
NT = (((1,), (1,)), ((), ()))

L = 128
TA = 256
NA = S // TA
HG = 8
NG = H // HG
HR = HG * DH
GR = 3 * HR
QD = D // 4
TF = 512
HF = TF // 2
NF = F // TF
UNITS = ((0, 4), (4, 2), (6, 2))
QS = ((0, 0), (0, 1), (1, 0), (1, 1))

WQ = ((0, 384), (512, 896), (1152, 1536), (384, 512), (896, 1152), (1536, 1728))
MOD_A, MOD_B = 2 * D, 2944

SORD = (4, 1, 0, 3, 2, 6, 5)
SIN = (((0, 0), (1, 1), 1), ((1, 0), (1, 1), 1), ((0, 0), None, 0), ((1, 1), None, 0),
       ((0, 0), (0, 1), 1), ((1, 0), (0, 0), -1), ((0, 1), (1, 1), -1))
SOUT = ((((0, 0), 1), ((1, 1), 1)), (((1, 0), 1), ((1, 1), -1)), (((0, 1), 1), ((1, 1), 1)),
        (((0, 0), 1), ((1, 0), 1)), (((0, 0), -1), ((0, 1), 1)), (((1, 1), 1),), (((0, 0), 1),))

LAM = (-2.0, -0.5, 0.5, 2.0)
PAIRS = tuple((i, j) for i in range(4) for j in range(i + 1, 4))
DORD = (4, 0, 5, 1, 8, 9, 10, 6, 2, 11, 12, 13, 17, 18, 19, 7, 3, 14, 15, 16, 20, 21, 22, 23, 24, 25)

C2 = 48
N_LN1 = 2 * (D // 16)
N_LN2A = 2 * (D // C2)
N_LN2B = 7 * 4


class _Ticker:
    def __init__(self, toks=None, n=1):
        self.toks, self.n, self.k = toks, n, 0

    def __call__(self):
        if not self.toks:
            return None
        tok = self.toks[min(self.k * len(self.toks) // self.n, len(self.toks) - 1)]
        self.k += 1
        return jnp.where(tok > jnp.inf, 1.0, 0.0)


class _Idx:
    def __init__(self, base, off=0):
        self.base, self.off = base, off

    def __add__(self, k):
        return _Idx(self.base, self.off + k)

    def __sub__(self, k):
        return _Idx(self.base, self.off - k)

    def __mod__(self, m):
        assert m == 2
        return self.off % 2

    def __rmul__(self, k):
        return k * self.base + k * self.off

    __mul__ = __rmul__


def _iv(i):
    return i.base + i.off if isinstance(i, _Idx) else i


def _toks(res):
    return [res[r:r + 8, t * L:(t + 1) * L]
            for t in range(res.shape[1] // L) for r in range(0, res.shape[0], 8)]


def _plus(v, tick):
    if tick is None:
        return v
    n = v.shape[1] // L
    return v + (tick if n == 1 else jnp.concatenate([tick] * n, axis=1))


def _stats(k8, s1, s2):
    md = jnp.sum(s1, axis=0, keepdims=True) * (1.0 / D)
    var = jnp.sum(s2, axis=0, keepdims=True) * (1.0 / D) - md * md
    rs = jax.lax.rsqrt(jnp.maximum(var, 0.0) + 1e-5)
    return k8 + md, jnp.broadcast_to(rs, k8.shape)


def _silu_mul(g, u):
    hg = 0.5 * g
    return (hg * jnp.tanh(hg) + hg) * u


def _sa(x11, x12, x21, x22):
    return [x11 + x22, x21 + x22, x11, x22, x11 + x12, x21 - x11, x12 - x22]


def _sb(y11, y12, y21, y22):
    return [y11 + y22, y11, y12 - y22, y21 - y11, y22, y11 + y12, y21 + y22]


def _strassen_out(get, cacc):
    cacc = dict(cacc)
    for a in range(7):
        p = [get(a, b) for b in range(7)]
        inn = {(0, 0): p[0] + p[3] - p[4] + p[6], (0, 1): p[2] + p[4],
               (1, 0): p[1] + p[3], (1, 1): p[0] - p[1] + p[2] + p[5]}
        for tgt, sign in SOUT[a]:
            for q in QS:
                cacc[tgt + q] = cacc[tgt + q] + inn[q] if sign > 0 else cacc[tgt + q] - inn[q]
    return cacc


def _hk_a(xy):
    def z(l, i):
        x, y = xy(l, i)
        return y + LAM[l] * x

    zd = [z(i, i) for i in range(4)]
    ops = [xy(i, i)[0] for i in range(4)] + zd
    for i, j in PAIRS:
        r = 1.0 / (LAM[i] - LAM[j])
        ops += [(zd[i] - zd[j]) * r, (z(j, i) - zd[j]) * r, (z(i, j) - zd[i]) * r]
    return ops


def _hk_b(b1, b2):
    u = [b1[i] - LAM[i] * b2[i] for i in range(4)]
    ops = u + list(b2)
    for i, j in PAIRS:
        ops += [u[i] + u[j], (u[i] + b1[j]) - LAM[i] * b2[j], (u[j] + b1[i]) - LAM[j] * b2[i]]
    return ops


def _hk_c_row(m, i, tick):
    p = _plus(m(i), tick)
    out = []
    for j in range(4):
        if j == i:
            out.append(p + m(4 + i))
        else:
            k = 8 + 3 * PAIRS.index((min(i, j), max(i, j)))
            v = (m(4 + j) - p) + m(k)
            out.append(v - m(k + 1) if i < j else v + m(k + 2))
    return out


def _pk(v):
    return pltpu.bitcast(v.astype(bf16), u32)


def _upk(v):
    return pltpu.bitcast(v, bf16)


def _kernel(x_hbm, c_hbm, wmod_hbm, wqkv_hbm, wo_hbm, w1_hbm, w3_hbm, w2t_hbm, out_hbm,
            c_v, x_v, wmod_v, wqkv_v, wqkvT, wo_v, woT, w1_v, w3_v, w2t_v,
            modb, modr, h_sc, q_sc, k_sc, v_sc, o_sc, x1_sc, st_sc, a_sc, t_sc, acc, out_v,
            sem):
    def cp_x(i):
        s = {1: 4, 2: 5}.get(i, 0)
        return pltpu.make_async_copy(x_hbm.at[:, pl.ds(i * TA, TA)], x_v.at[i], sem.at[s])

    def cp_f(k, j):
        src, dst = ((w1_hbm, w1_v), (w3_hbm, w3_v), (w2t_hbm, w2t_v))[k]
        return pltpu.make_async_copy(src.at[:, pl.ds(j * TF, TF)], dst.at[j], sem.at[2])

    def cp_cols(src, dst, lo, hi, s):
        return pltpu.make_async_copy(src.at[:, pl.ds(lo, hi - lo)], dst.at[:, pl.ds(lo, hi - lo)], sem.at[s])

    def cp_wq(k):
        return cp_cols(wqkv_hbm, wqkv_v, WQ[k][0], WQ[k][1], min(1 + k, 4))

    def cp_o(ii, ri):
        rows = pl.ds(ri * QD, QD)
        return pltpu.make_async_copy(out_v.at[ii, rows], out_hbm.at[rows, pl.ds(ii * 2 * TA, 2 * TA)],
                                     sem.at[3])

    cp_moda = cp_cols(wmod_hbm, wmod_v, 0, MOD_A, 0)
    cp_modb = cp_cols(wmod_hbm, wmod_v, MOD_A, MOD_B, 5)
    cp_modc = cp_cols(wmod_hbm, wmod_v, MOD_B, 6 * D, 2)
    cp_c = pltpu.make_async_copy(c_hbm, c_v, sem.at[0])
    cp_wo = pltpu.make_async_copy(wo_hbm, wo_v, sem.at[5])

    cp_moda.start()
    cp_x(0).start()
    cp_c.start()
    for cp in [cp_wq(k) for k in range(6)] + [cp_x(1), cp_wo, cp_modb, cp_x(2)]:
        cp.start(priority=1)

    acc[...] = jnp.zeros(acc.shape, f32)
    k_sc[0] = jnp.zeros(k_sc.shape[1:], u32)
    v_sc[0] = jnp.zeros(v_sc.shape[1:], f32)

    def mod_cols(lo, hi):
        c = c_v[...].astype(f32)
        sc = jnp.broadcast_to((c * jax.nn.sigmoid(c)).astype(bf16), (16, D))
        return jnp.dot(sc, wmod_v[:, lo:hi], preferred_element_type=f32)[0:8]

    def col_bcast(row):
        return jnp.broadcast_to(row[0:1], (L, D)).T

    def tr_wq(k):
        lo, hi = WQ[k]
        wt = pltpu.bitcast(wqkv_v[:, lo:hi].T, u32)
        c = lo
        while c < hi:
            e = min(hi, (c // HR + 1) * HR)
            dst = (c % D) // HR * GR + c // D * HR + c % HR
            wqkvT[dst // 2:(dst + e - c) // 2, :] = wt[(c - lo) // 2:(e - lo) // 2, :]
            c = e

    def ln1(i, i2, slot, tk):
        k8 = jnp.broadcast_to(x_v[i, 0:16, :].astype(f32)[0:1], (8, TA))
        s1 = s2 = None
        for r in range(0, D, 16):
            kk = _plus(k8, tk())
            x = x_v[i, r:r + 16, :].astype(f32)
            for h in range(2):
                d = x[8 * h:8 * h + 8] - kk
                s1 = d if s1 is None else s1 + d
                s2 = d * d if s2 is None else s2 + d * d
        m8, rs8 = _stats(k8, s1, s2)
        for r in range(0, D, 16):
            mk = _plus(m8, tk())
            x = x_v[i2, r:r + 16, :].astype(f32)
            rows = []
            for h in range(2):
                rr = slice(r + 8 * h, r + 8 * h + 8)
                xn = (x[8 * h:8 * h + 8] - mk) * rs8
                rows.append(jnp.concatenate(
                    [xn[:, t * L:(t + 1) * L] * modb[1, rr] + modb[0, rr] for t in range(2)], axis=1))
            h_sc[slot, r // 2:r // 2 + 8] = _pk(jnp.concatenate(rows, axis=0))

    def qkv_part(i, u, hooks=None):
        h = _upk(h_sc[i % 2])
        toks, res = [], []
        for r in range(3):
            lo = (u * GR + r * HR) // 2
            res.append(jnp.dot(_upk(wqkvT[lo:lo + HR // 2, :]), h, preferred_element_type=f32))
            toks += _toks(res[r])
            if hooks:
                hooks.pop(0)()
        for t in range(2):
            q_sc[t, u] = res[0][:, t * L:(t + 1) * L]
            k_sc[2 * i + t + 1, u] = _pk(res[1][:, t * L:(t + 1) * L])
            v_sc[2 * i + t + 1, u] = res[2][:, t * L:(t + 1) * L]
        return toks

    def attn(i, u):
        lane = jax.lax.broadcasted_iota(jnp.int32, (HG, L), 1)

        def shift(cur, prev, w):
            return pltpu.roll(jnp.where(lane < L - DIL * w, cur, prev), DIL * w, 1)

        def weights(t):
            g = 2 * i + t
            lg = [None] * W
            for p in range(DH // 2):
                q0 = q_sc[t, u, pl.ds(2 * p, HG, stride=DH), :]
                q1 = q_sc[t, u, pl.ds(2 * p + 1, HG, stride=DH), :]
                cur = k_sc[g + 1, u, pl.ds(p, HG, stride=DH // 2), :]
                prev = k_sc[g, u, pl.ds(p, HG, stride=DH // 2), :]
                for w in range(W):
                    kw = cur if w == 0 else shift(cur, prev, w)
                    k0 = pltpu.bitcast(kw << 16, f32)
                    k1 = pltpu.bitcast(kw & jnp.uint32(0xFFFF0000), f32)
                    tmp = q0 * k0 + q1 * k1
                    lg[w] = tmp if lg[w] is None else lg[w] + tmp
            pos = lane + g * L
            lg = [v * (DH ** -0.5) for v in lg]
            for w in range(1, W):
                lg[w] = jnp.where(pos >= DIL * w, lg[w], -1e9)
            m = lg[0]
            for w in range(1, W):
                m = jnp.maximum(m, lg[w])
            es = [jnp.exp(v - m) for v in lg]
            den = es[0]
            for w in range(1, W):
                den = den + es[w]
            inv = 1.0 / den
            return [e * inv for e in es]

        def values(t, at):
            g = 2 * i + t
            for d in range(DH):
                cur = v_sc[g + 1, u, pl.ds(d, HG, stride=DH), :]
                prev = v_sc[g, u, pl.ds(d, HG, stride=DH), :]
                o = at[0] * cur
                for w in range(1, W):
                    o = o + at[w] * shift(cur, prev, w)
                o_sc[i % 2, t, pl.ds(u * HR + d, HG, stride=DH), :] = o

        ats = [weights(t) for t in range(2)]
        for t in range(2):
            values(t, ats[t])

    def wo_res(i):
        o = jnp.concatenate([o_sc[i % 2, 0], o_sc[i % 2, 1]], axis=1).astype(bf16)
        mo = D // 2
        k8, s1, s2 = [None] * 2, [None] * 2, [None] * 2
        toks = []
        for r in range(2):
            att = jnp.dot(_upk(woT[r * mo // 2:(r + 1) * mo // 2, :]), o, preferred_element_type=f32)
            toks += _toks(att)
            rs = slice(r * mo, (r + 1) * mo)
            x = x_v[_iv(i), rs, :].astype(f32)
            for t in range(2):
                x1 = x[:, t * L:(t + 1) * L] + att[:, t * L:(t + 1) * L]
                x1_sc[2 * i + t, rs] = x1
                if r == 0:
                    k8[t] = jnp.broadcast_to(x1[0:1], (8, L))
                for q in range(0, mo, 8):
                    d = x1[q:q + 8] - k8[t]
                    s1[t] = d if s1[t] is None else s1[t] + d
                    s2[t] = d * d if s2[t] is None else s2[t] + d * d
        for t in range(2):
            st_sc[2 * i + t, 0], st_sc[2 * i + t, 1], st_sc[2 * i + t, 2] = k8[t], s1[t], s2[t]
        return toks

    def ln2a(i, tk):
        h2 = []
        for t in range(2):
            m8, rs8 = _stats(st_sc[2 * i + t, 0], st_sc[2 * i + t, 1], st_sc[2 * i + t, 2])
            rows = []
            for r in range(0, D, 8):
                if r % C2 == 0:
                    mk = _plus(m8, tk())
                rows.append((x1_sc[2 * i + t, r:r + 8] - mk) * rs8)
            h2.append(jnp.concatenate(rows, axis=0).T * modr[1, 0:1] + modr[0, 0:1])
        return h2

    def ln2b(i, h2, tk):
        r0 = i * 32 if isinstance(i, int) else pl.multiple_of(i * 32, 32)
        for a1, a2 in QS:
            t_sc[2 * a1 + a2, pl.ds(r0, 32), :] = _pk(h2[a1][64 * a2:64 * a2 + 64, 512:D])
        blk = ((h2[0][:, 0:256], h2[0][:, 256:512]), (h2[1][:, 0:256], h2[1][:, 256:512]))
        for a in (2, 4, 5, 0, 1, 3, 6):
            p0, p1, sgn = SIN[a]
            for r in range(0, 64, 16):
                tick = tk()
                xs = []
                for a2 in range(2):
                    rows = []
                    for q in range(64 * a2 + r, 64 * a2 + r + 16, 8):
                        v = _plus(blk[p0[0]][p0[1]][q:q + 8], tick)
                        if p1 is not None:
                            o = blk[p1[0]][p1[1]][q:q + 8]
                            v = v + o if sgn > 0 else v - o
                        rows.append(v)
                    xs.append(jnp.concatenate(rows, axis=0))
                for b, v in enumerate(_sa(xs[0][:, 0:L], xs[0][:, L:], xs[1][:, 0:L], xs[1][:, L:])):
                    a_sc[7 * a + b, pl.ds(r0 + r // 2, 8), :] = _pk(v)

    notick = _Ticker()
    cp_c.wait()
    cp_moda.wait()
    cp_x(0).wait()
    mod = mod_cols(0, MOD_A)
    modb[0] = col_bcast(mod[:, 0:D])
    modb[1] = col_bcast(mod[:, D:2 * D] + 1.0)
    ln1(0, 0, 0, notick)

    for k in range(3):
        cp_wq(k).wait()
        tr_wq(k)
    qkv_part(0, 0)
    qkv_part(0, 1)
    attn(0, 0)

    for k in range(3, 6):
        cp_wq(k).wait()
    cp_x(1).wait()
    for k in range(3, 6):
        tr_wq(k)
    toks = []
    for u in range(2, NG):
        toks += qkv_part(0, u)
        attn(0, u - 1)
    ln1(1, 1, 1, _Ticker(toks[0:150], N_LN1))
    for u in range(NG - 1):
        qkv_part(1, u)
        if u == 0:
            attn(0, NG - 1)
        else:
            attn(1, u - 1)

    cp_wo.wait()
    cp_modb.wait()
    cp_x(2).wait()
    for i in range(3, NA):
        cp_x(i).start()
    cp_modc.start(priority=1)
    for j in range(NF):
        for k in range(3):
            cp_f(k, j).start(priority=1)
    pieces = []
    cuts = [MOD_A + v * L for v in (0, 5, 8, 11)] + [MOD_B]
    hooks = [(lambda lo=lo, hi=hi: pieces.append(mod_cols(lo, hi))) for lo, hi in zip(cuts, cuts[1:])]
    hooks.pop(0)()
    toks = qkv_part(1, NG - 1, hooks)
    attn(1, NG - 2)
    mod = jnp.concatenate(pieces, axis=1)
    woT[...] = pltpu.bitcast((wo_v[...].astype(f32) * mod[0:1, 0:D]).astype(bf16).T, u32)
    modr[0] = mod[:, D:2 * D]
    modr[1] = mod[:, 2 * D:3 * D] + 1.0
    toks += wo_res(0)
    attn(1, NG - 1)
    ln1(2, 2, 0, _Ticker(toks[len(toks) // 4:-16], N_LN1))

    for i in range(3, NA):
        cp_x(i).wait()

    def a_tile(i):
        toks = []
        for u in range(NG):
            toks += qkv_part(i, u)
            if u > 0:
                attn(i, u - 1)
        h2 = ln2a(i - 2, notick)
        toks += wo_res(i - 1)
        attn(i, NG - 1)
        ln2b(i - 2, h2, _Ticker(toks[20:108] + toks[490:570], N_LN2B))
        ln1(jnp.minimum(_iv(i) + 1, NA - 1), jnp.minimum(_iv(i), NA - 2) + 1, (i + 1) % 2,
            _Ticker(toks[108:500], N_LN1))

    def a_body(it, carry):
        for d in range(2):
            a_tile(_Idx(2 + 2 * it, d))
        return carry

    jax.lax.fori_loop(0, (NA - 2) // 2, a_body, 0)

    cp_modc.wait()
    for j in range(NF):
        for k in range(3):
            cp_f(k, j).wait()
    modb[2] = col_bcast(mod_cols(MOD_B - L, 6 * D)[:, 5 * D - (MOD_B - L):])
    toks = wo_res(NA - 1)
    ln2b(NA - 2, ln2a(NA - 2, notick), _Ticker(toks[0:100], N_LN2B))

    def fin(ii, ri, tk):
        cs = slice(ii * L, (ii + 1) * L)
        lo = jax.lax.broadcasted_iota(jnp.int32, (8, L), 1) < 64
        for r in range(0, QD, 8):
            cc = _hk_c_row(lambda k: acc[k, r:r + 8, cs], ri, tk())
            rows = slice(ri * QD + r, ri * QD + r + 8)
            res = [[], []]
            for a1 in range(2):
                v0, v1 = cc[2 * a1], cc[2 * a1 + 1]
                z = pltpu.roll(jnp.where(lo, v1, v0), 64, 1)
                for par, v in enumerate((jnp.where(lo, v0, z), jnp.where(lo, z, v1))):
                    res[par].append(x1_sc[2 * (2 * ii + par) + a1, rows] + modb[2, rows] * v)
            out_v[ii, rows, :] = jnp.concatenate(res[0] + res[1], axis=1).astype(bf16)

    def b_body(j, carry):
        js = (j, jnp.minimum(j, NF - 1), jnp.maximum(j, 0), jnp.clip(j, 0, NF - 1))
        bw = {}
        for c1, wv in enumerate((w1_v, w3_v)):
            for a in SORD:
                jj = js[(0, 1, 1, 2, 2, 3, 3)[a]]
                y = _sb(wv[jj, 0:256, 0:HF].astype(f32), wv[jj, 0:256, HF:TF].astype(f32),
                        wv[jj, 256:512, 0:HF].astype(f32), wv[jj, 256:512, HF:TF].astype(f32))[a]
                for b, v in enumerate(_sb(y[0:L, 0:L], y[0:L, L:], y[L:, 0:L], y[L:, L:])):
                    bw[(c1, a, b)] = v.astype(bf16)
        aw = [v.astype(bf16) for v in _hk_a(lambda l, i: (
            w2t_v[js[l], i * QD:(i + 1) * QD, 0:HF].astype(f32),
            w2t_v[js[l], i * QD:(i + 1) * QD, HF:TF].astype(f32)))]

        def gate_up(tt):
            t0, nt = UNITS[tt]
            rq = slice(t0 * 32, (t0 + nt) * 32)
            main, rem = {}, {}
            for c1 in range(2):
                for a in SORD:
                    for b in SORD:
                        main[(c1, a, b)] = jnp.dot(_upk(a_sc[7 * a + b, rq, :]), bw[(c1, a, b)],
                                                   preferred_element_type=f32)
            for a1, a2 in QS:
                for c2, nn in QS:
                    for c1, wv in enumerate((w1_v, w3_v)):
                        col = c2 * HF + nn * L
                        rem[(c1, a1, c2, a2, nn)] = jnp.dot(
                            _upk(t_sc[2 * a1 + a2, rq, :]), wv[j, 512:D, col:col + L],
                            preferred_element_type=f32)
            keep = lambda v: jnp.concatenate([v[0:64], v[64:]], axis=0)
            g, u = [_strassen_out(lambda a, b: keep(main[(c1, a, b)]),
                                  {k1 + k2: keep(rem[(c1,) + k1 + k2]) for k1 in QS for k2 in QS})
                    for c1 in range(2)]
            act = {k: _silu_mul(g[k], u[k]) for k in g}
            blk = lambda a1, a2, c2: jnp.concatenate([act[(a1, c2, a2, nn)] for nn in range(2)], axis=1)
            eb = [v.astype(bf16) for v in _hk_b([blk(a1, a2, 0) for a1, a2 in QS],
                                                [blk(a1, a2, 1) for a1, a2 in QS])]
            return eb, list(main.values())

        def down(tt, eb):
            t0, nt = UNITS[tt]
            res = []
            for k in DORD:
                d = jax.lax.dot_general(aw[k], eb[k], NT, preferred_element_type=f32)
                acc[k, :, t0 * 64:(t0 + nt) * 64] += d
                res.append(d)
            return res

        def finish(tt, prods):
            t0, nt = UNITS[tt]
            toks = [v[r:r + 8, 0:L] for v in prods for r in range(0, v.shape[0], 16)]
            tk = _Ticker(toks, 2 * nt * (QD // 8))
            for ii in range(t0 // 2, (t0 + nt) // 2):
                for ri in range(4):
                    fin(ii, ri, tk)

                    @pl.when(j == NF - 1)
                    def _():
                        cp_o(ii, ri).start()

        eb0, _ = gate_up(0)
        eb1, prods = gate_up(1)
        gt = [v[r:r + 8] for v in prods for r in range(0, v.shape[0], 32)]
        n = len(gt)
        ln2b(NA - 1, ln2a(NA - 1, _Ticker(gt[n * 5 // 100:n * 30 // 100], N_LN2A)),
             _Ticker(gt[n * 35 // 100:n * 95 // 100], N_LN2B))
        down(0, eb0)
        eb2, prods = gate_up(2)
        finish(0, prods[0:92])
        down(1, eb1)
        finish(1, down(2, eb2)[0:24])
        return carry

    jax.lax.fori_loop(0, NF, b_body, 0)

    for ri in range(4):
        fin(NA // 2 - 1, ri, notick)
        cp_o(NA // 2 - 1, ri).start()
    for ii in range(NA // 2):
        for ri in range(4):
            cp_o(ii, ri).wait()


@jax.jit
def pallas_adaLN_cond__sliding_local_dilated__glu_gated_swiglu__prompt_kernel(
    A_x: jax.Array,
    A_wqkv: jax.Array,
    A_wo: jax.Array,
    B_x: jax.Array,
    B_w1: jax.Array,
    B_w3: jax.Array,
    B_w2: jax.Array,
    c: jax.Array,
    w_mod: jax.Array,
):
    del B_x
    hbm = pl.BlockSpec(memory_space=pl.ANY)
    out_t = pl.pallas_call(
        _kernel,
        in_specs=[hbm] * 8,
        out_specs=hbm,
        out_shape=jax.ShapeDtypeStruct((D, S), bf16),
        scratch_shapes=[
            pltpu.VMEM((1, D), bf16),
            pltpu.VMEM((NA, D, TA), bf16),
            pltpu.VMEM((D, 6 * D), bf16),
            pltpu.VMEM((D, 3 * D), bf16),
            pltpu.VMEM((3 * D // 2, D), u32),
            pltpu.VMEM((D, D), bf16),
            pltpu.VMEM((D // 2, D), u32),
            pltpu.VMEM((NF, D, TF), bf16),
            pltpu.VMEM((NF, D, TF), bf16),
            pltpu.VMEM((NF, D, TF), bf16),
            pltpu.VMEM((3, D, L), f32),
            pltpu.VMEM((2, 8, D), f32),
            pltpu.VMEM((2, D // 2, TA), u32),
            pltpu.VMEM((2, NG, HR, L), f32),
            pltpu.VMEM((2 * NA + 1, NG, HR // 2, L), u32),
            pltpu.VMEM((2 * NA + 1, NG, HR, L), f32),
            pltpu.VMEM((2, 2, D, L), f32),
            pltpu.VMEM((2 * NA, D, L), f32),
            pltpu.VMEM((2 * NA, 3, 8, L), f32),
            pltpu.VMEM((49, S // 8, L), u32),
            pltpu.VMEM((4, S // 8, 64), u32),
            pltpu.VMEM((26, QD, S // 4), f32),
            pltpu.VMEM((NA // 2, D, 2 * TA), bf16),
            pltpu.SemaphoreType.DMA((6,)),
        ],
        compiler_params=pltpu.CompilerParams(vmem_limit_bytes=100 * 1024 * 1024),
    )(A_x.reshape(S, D).T, c, w_mod, A_wqkv, A_wo, B_w1, B_w3, B_w2.T)
    return out_t.T.reshape(1, S, D)
```

```python
import jax
import jax.numpy as jnp
import jax.experimental.pallas as pl
import jax.experimental.pallas.tpu as pltpu

S, D, F, H, DH, W, DIL = 2048, 576, 4608, 32, 18, 8, 2
f32 = jnp.float32
bf16 = jnp.bfloat16
u32 = jnp.uint32
NT = (((1,), (1,)), ((), ()))

L = 128
TA = 256
NA = S // TA
HG = 8
NG = H // HG
HR = HG * DH
GR = 3 * HR
QD = D // 4
TF = 512
HF = TF // 2
NF = F // TF
UNITS = ((0, 4), (4, 2), (6, 2))
QS = ((0, 0), (0, 1), (1, 0), (1, 1))

WQ = ((0, 384), (512, 896), (1152, 1536), (384, 512), (896, 1152), (1536, 1728))
MOD_A, MOD_B = 2 * D, 2944

SORD = (4, 1, 0, 3, 2, 6, 5)
SIN = (((0, 0), (1, 1), 1), ((1, 0), (1, 1), 1), ((0, 0), None, 0), ((1, 1), None, 0),
       ((0, 0), (0, 1), 1), ((1, 0), (0, 0), -1), ((0, 1), (1, 1), -1))
SRIN = (((0, 0), (1, 1), 1), ((0, 0), None, 0), ((0, 1), (1, 1), -1), ((1, 0), (0, 0), -1),
        ((1, 1), None, 0), ((0, 0), (0, 1), 1), ((1, 0), (1, 1), 1))
SOUT = ((((0, 0), 1), ((1, 1), 1)), (((1, 0), 1), ((1, 1), -1)), (((0, 1), 1), ((1, 1), 1)),
        (((0, 0), 1), ((1, 0), 1)), (((0, 0), -1), ((0, 1), 1)), (((1, 1), 1),), (((0, 0), 1),))

LAM = (-2.0, -0.5, 0.5, 2.0)
PAIRS = tuple((i, j) for i in range(4) for j in range(i + 1, 4))
DORD = (4, 0, 5, 1, 8, 9, 10, 6, 2, 11, 12, 13, 17, 18, 19, 7, 3, 14, 15, 16, 20, 21, 22, 23, 24, 25)

C2 = 48
N_LN1 = 2 * (D // 16)
N_LN2A = 2 * (D // C2)
N_LN2B = 7 * 4


class _Ticker:
    def __init__(self, toks=None, n=1):
        self.toks, self.n, self.k = toks, n, 0

    def __call__(self):
        if not self.toks:
            return None
        res, r, c = self.toks[min(self.k * len(self.toks) // self.n, len(self.toks) - 1)]
        self.k += 1
        return jnp.where(res[r:r + 8, c:c + L] > jnp.inf, 1.0, 0.0)


class _Idx:
    def __init__(self, base, off=0):
        self.base, self.off = base, off

    def __add__(self, k):
        return _Idx(self.base, self.off + k)

    def __sub__(self, k):
        return _Idx(self.base, self.off - k)

    def __mod__(self, m):
        assert m == 2
        return self.off % 2

    def __rmul__(self, k):
        return k * self.base + k * self.off

    __mul__ = __rmul__


def _iv(i):
    return i.base + i.off if isinstance(i, _Idx) else i


def _toks(res, step=8, cols=None):
    return [(res, r, c) for c in range(0, cols or res.shape[1], L) for r in range(0, res.shape[0], step)]


def _plus(v, tick):
    if tick is None:
        return v
    n = v.shape[1] // L
    return v + (tick if n == 1 else jnp.concatenate([tick] * n, axis=1))


def _g8(v):
    return v.reshape(v.shape[0] // 8, 8, v.shape[1])


def _stack(tiles):
    return _g8(jnp.concatenate(tiles, axis=0))


def _ticks(tk, n, rep=1):
    ts = [tk() for _ in range(n)]
    if ts[0] is None:
        return None
    return jnp.concatenate([t for t in ts for _ in range(rep)], axis=0)


def _rows(v8, tk, n, rep):
    return _stack([v for v in [_plus(v8, tk()) for _ in range(n)] for _ in range(rep)])


def _stats(k8, s1, s2):
    md = jnp.sum(s1, axis=0, keepdims=True) * (1.0 / D)
    var = jnp.sum(s2, axis=0, keepdims=True) * (1.0 / D) - md * md
    rs = jax.lax.rsqrt(jnp.maximum(var, 0.0) + 1e-5)
    return k8 + md, jnp.broadcast_to(rs, k8.shape)


def _silu_mul(g, u):
    hg = 0.5 * g
    return (hg * jnp.tanh(hg) + hg) * u


def _sa(x11, x12, x21, x22):
    return [x11 + x22, x21 + x22, x11, x22, x11 + x12, x21 - x11, x12 - x22]


def _sb(y11, y12, y21, y22):
    return [y11 + y22, y11, y12 - y22, y21 - y11, y22, y11 + y12, y21 + y22]


def _strassen_out(get, cacc):
    cacc = dict(cacc)
    for a in range(7):
        p = [get(a, b) for b in range(7)]
        inn = {(0, 0): p[0] + p[3] - p[4] + p[6], (0, 1): p[2] + p[4],
               (1, 0): p[1] + p[3], (1, 1): p[0] - p[1] + p[2] + p[5]}
        for tgt, sign in SOUT[a]:
            for q in QS:
                cacc[tgt + q] = cacc[tgt + q] + inn[q] if sign > 0 else cacc[tgt + q] - inn[q]
    return cacc


def _hk_a(xy):
    def z(l, i):
        x, y = xy(l, i)
        return y + LAM[l] * x

    zd = [z(i, i) for i in range(4)]
    ops = [xy(i, i)[0] for i in range(4)] + zd
    for i, j in PAIRS:
        r = 1.0 / (LAM[i] - LAM[j])
        ops += [(zd[i] - zd[j]) * r, (z(j, i) - zd[j]) * r, (z(i, j) - zd[i]) * r]
    return ops


def _hk_b(b1, b2):
    u = [b1[i] - LAM[i] * b2[i] for i in range(4)]
    ops = u + list(b2)
    for i, j in PAIRS:
        ops += [u[i] + u[j], (u[i] + b1[j]) - LAM[i] * b2[j], (u[j] + b1[i]) - LAM[j] * b2[i]]
    return ops


def _hk_c_row(m, i, tick):
    p = _plus(m(i), tick)
    out = []
    for j in range(4):
        if j == i:
            out.append(p + m(4 + i))
        else:
            k = 8 + 3 * PAIRS.index((min(i, j), max(i, j)))
            v = (m(4 + j) - p) + m(k)
            out.append(v - m(k + 1) if i < j else v + m(k + 2))
    return out


def _pk(v):
    return pltpu.bitcast(v.astype(bf16), u32)


def _upk(v):
    return pltpu.bitcast(v, bf16)


def _kernel(x_hbm, c_hbm, wmod_hbm, wqkv_hbm, wo_hbm, w1_hbm, w3_hbm, w2t_hbm, out_hbm,
            c_v, x_v, wmod_v, wqkv_v, wqkvT, wo_v, woT, w1_v, w3_v, w2t_v,
            modb, modr, h_sc, q_sc, k_sc, v_sc, o_sc, x1_sc, st_sc, a_sc, t_sc, acc, out_v,
            sem):
    def cp_x(i):
        s = {1: 4, 2: 5}.get(i, 0)
        return pltpu.make_async_copy(x_hbm.at[:, pl.ds(i * TA, TA)], x_v.at[i], sem.at[s])

    def cp_f(k, j):
        src, dst = ((w1_hbm, w1_v), (w3_hbm, w3_v), (w2t_hbm, w2t_v))[k]
        return pltpu.make_async_copy(src.at[:, pl.ds(j * TF, TF)], dst.at[j], sem.at[2])

    def cp_cols(src, dst, lo, hi, s):
        return pltpu.make_async_copy(src.at[:, pl.ds(lo, hi - lo)], dst.at[:, pl.ds(lo, hi - lo)], sem.at[s])

    def cp_wq(k):
        return cp_cols(wqkv_hbm, wqkv_v, WQ[k][0], WQ[k][1], min(1 + k, 4))

    def cp_o(ii, ri):
        rows = pl.ds(ri * QD, QD)
        return pltpu.make_async_copy(out_v.at[ii, rows], out_hbm.at[rows, pl.ds(ii * 2 * TA, 2 * TA)],
                                     sem.at[3])

    cp_moda = cp_cols(wmod_hbm, wmod_v, 0, MOD_A, 0)
    cp_modb = cp_cols(wmod_hbm, wmod_v, MOD_A, MOD_B, 5)
    cp_modc = cp_cols(wmod_hbm, wmod_v, MOD_B, 6 * D, 2)
    cp_c = pltpu.make_async_copy(c_hbm, c_v, sem.at[0])
    cp_wo = pltpu.make_async_copy(wo_hbm, wo_v, sem.at[5])

    cp_moda.start()
    cp_x(0).start()
    cp_c.start()
    for cp in [cp_wq(k) for k in range(6)] + [cp_x(1), cp_wo, cp_modb, cp_x(2)]:
        cp.start(priority=1)

    acc[...] = jnp.zeros(acc.shape, f32)
    k_sc[0] = jnp.zeros(k_sc.shape[1:], u32)
    v_sc[0] = jnp.zeros(v_sc.shape[1:], f32)

    def mod_cols(lo, hi):
        c = c_v[...].astype(f32)
        sc = jnp.broadcast_to((c * jax.nn.sigmoid(c)).astype(bf16), (16, D))
        return jnp.dot(sc, wmod_v[:, lo:hi], preferred_element_type=f32)[0:8]

    def col_bcast(row):
        return jnp.broadcast_to(row[0:1], (L, D)).T

    def tr_wq(k):
        lo, hi = WQ[k]
        wt = pltpu.bitcast(wqkv_v[:, lo:hi].T, u32)
        c = lo
        while c < hi:
            e = min(hi, (c // HR + 1) * HR)
            dst = (c % D) // HR * GR + c // D * HR + c % HR
            wqkvT[dst // 2:(dst + e - c) // 2, :] = wt[(c - lo) // 2:(e - lo) // 2, :]
            c = e

    def ln1(i, i2, slot, tk):
        k8 = jnp.broadcast_to(x_v[i, 0:16, :].astype(f32)[0:1], (8, TA))
        d = _g8(x_v[i].astype(f32)) - _rows(k8, tk, D // 16, 2)
        m8, rs8 = _stats(k8, jnp.sum(d, axis=0), jnp.sum(d * d, axis=0))
        xn = ((_g8(x_v[i2].astype(f32)) - _rows(m8, tk, D // 16, 2)) * rs8).reshape(D, TA)
        h_sc[slot] = _pk(jnp.concatenate(
            [xn[:, t * L:(t + 1) * L] * modb[1] + modb[0] for t in range(2)], axis=1))

    def qkv_part(i, u, hooks=None):
        h = _upk(h_sc[i % 2])
        toks, res = [], []
        for r in range(3):
            lo = (u * GR + r * HR) // 2
            res.append(jnp.dot(_upk(wqkvT[lo:lo + HR // 2, :]), h, preferred_element_type=f32))
            toks += _toks(res[r])
            if hooks:
                hooks.pop(0)()
        for t in range(2):
            q_sc[t, u] = res[0][:, t * L:(t + 1) * L]
            k_sc[2 * i + t + 1, u] = _pk(res[1][:, t * L:(t + 1) * L])
            v_sc[2 * i + t + 1, u] = res[2][:, t * L:(t + 1) * L]
        return toks

    lane = jax.lax.broadcasted_iota(jnp.int32, (HG, L), 1)

    def attn(i, u):
        keep = [lane < L - DIL * w for w in range(W)]

        def windows(ref, g, p, stride):
            cur = ref[g + 1, u, pl.ds(p, HG, stride=stride), :]
            prev = ref[g, u, pl.ds(p, HG, stride=stride), :]
            return _stack([cur] + [pltpu.roll(jax.lax.select(keep[w], cur, prev), DIL * w, 1)
                                   for w in range(1, W)])

        def weights(t):
            g = 2 * i + t
            lg = None
            for p in range(DH // 2):
                q0 = q_sc[t, u, pl.ds(2 * p, HG, stride=DH), :]
                q1 = q_sc[t, u, pl.ds(2 * p + 1, HG, stride=DH), :]
                kw = windows(k_sc, g, p, DH // 2)
                tmp = (q0 * pltpu.bitcast(kw << 16, f32)
                       + q1 * pltpu.bitcast(kw & jnp.uint32(0xFFFF0000), f32))
                lg = tmp if lg is None else lg + tmp
            lg = lg * (DH ** -0.5)
            pos = lane + g * L
            lg = _stack([lg[0]] + [jnp.where(pos >= DIL * w, lg[w], -1e9) for w in range(1, W)])
            e = jnp.exp(lg - jnp.max(lg, axis=0))
            return e * (1.0 / jnp.sum(e, axis=0))

        def values(t, at):
            for d in range(DH):
                o_sc[i % 2, t, pl.ds(u * HR + d, HG, stride=DH), :] = jnp.sum(
                    at * windows(v_sc, 2 * i + t, d, DH), axis=0)

        ats = [weights(t) for t in range(2)]
        for t in range(2):
            values(t, ats[t])

    def wo_res(i):
        o = jnp.concatenate([o_sc[i % 2, 0], o_sc[i % 2, 1]], axis=1).astype(bf16)
        mo = D // 2
        toks, x1 = [], []
        for r in range(2):
            att = jnp.dot(_upk(woT[r * mo // 2:(r + 1) * mo // 2, :]), o, preferred_element_type=f32)
            toks += _toks(att)
            x1.append(x_v[_iv(i), r * mo:(r + 1) * mo, :].astype(f32)
                      + jnp.concatenate([att[:, 0:L], att[:, L:]], axis=1))
        x1 = jnp.concatenate(x1, axis=0)
        k8 = jnp.broadcast_to(x1[0:1], (8, TA))
        d = _g8(x1) - k8
        st_sc[_iv(i), 0], st_sc[_iv(i), 1], st_sc[_iv(i), 2] = k8, jnp.sum(d, axis=0), jnp.sum(d * d, axis=0)
        for t in range(2):
            x1_sc[2 * i + t] = x1[:, t * L:(t + 1) * L]
        return toks

    def ln2a(i, tk):
        m8, rs8 = _stats(st_sc[_iv(i), 0], st_sc[_iv(i), 1], st_sc[_iv(i), 2])
        h2 = []
        for t in range(2):
            cs = slice(t * L, (t + 1) * L)
            xn = (_g8(x1_sc[2 * i + t]) - _rows(m8[:, cs], tk, D // C2, C2 // 8)) * rs8[:, cs]
            h2.append(xn.reshape(D, L).T * modr[1, 0:1] + modr[0, 0:1])
        return h2

    def ln2b(i, h2, tk):
        r0 = i * 32 if isinstance(i, int) else pl.multiple_of(i * 32, 32)
        for a1, a2 in QS:
            t_sc[2 * a1 + a2, pl.ds(r0, 32), :] = _pk(h2[a1][64 * a2:64 * a2 + 64, 512:D])
        blk = ((h2[0][:, 0:256], h2[0][:, 256:512]), (h2[1][:, 0:256], h2[1][:, 256:512]))
        for a in (2, 4, 5, 0, 1, 3, 6):
            p0, p1, sgn = SIN[a]
            tick = _ticks(tk, 4, 2)
            x = _plus(blk[p0[0]][p0[1]], None if tick is None else jnp.concatenate([tick, tick], axis=0))
            if p1 is not None:
                x = x + blk[p1[0]][p1[1]] if sgn > 0 else x - blk[p1[0]][p1[1]]
            for b, v in enumerate(_sa(x[0:64, 0:L], x[0:64, L:], x[64:, 0:L], x[64:, L:])):
                a_sc[7 * a + b, pl.ds(r0, 32), :] = _pk(v)

    notick = _Ticker()
    cp_c.wait()
    cp_moda.wait()
    cp_x(0).wait()
    mod = mod_cols(0, MOD_A)
    modb[0] = col_bcast(mod[:, 0:D])
    modb[1] = col_bcast(mod[:, D:2 * D] + 1.0)
    ln1(0, 0, 0, notick)

    for k in range(3):
        cp_wq(k).wait()
        tr_wq(k)
    qkv_part(0, 0)
    qkv_part(0, 1)
    attn(0, 0)

    for k in range(3, 6):
        cp_wq(k).wait()
    cp_x(1).wait()
    for k in range(3, 6):
        tr_wq(k)
    toks = []
    for u in range(2, NG):
        toks += qkv_part(0, u)
        attn(0, u - 1)
    ln1(1, 1, 1, _Ticker(toks[18:150], N_LN1))
    for u in range(NG - 1):
        qkv_part(1, u)
        if u == 0:
            attn(0, NG - 1)
        else:
            attn(1, u - 1)

    cp_wo.wait()
    cp_modb.wait()
    cp_x(2).wait()
    for i in range(3, NA):
        cp_x(i).start()
    cp_modc.start(priority=1)
    for j in range(NF):
        for k in range(3):
            cp_f(k, j).start(priority=1)
    pieces = []
    cuts = [MOD_A + v * L for v in (0, 5, 8, 11)] + [MOD_B]
    hooks = [(lambda lo=lo, hi=hi: pieces.append(mod_cols(lo, hi))) for lo, hi in zip(cuts, cuts[1:])]
    hooks.pop(0)()
    toks = qkv_part(1, NG - 1, hooks)
    attn(1, NG - 2)
    mod = jnp.concatenate(pieces, axis=1)
    woT[...] = pltpu.bitcast((wo_v[...].astype(f32) * mod[0:1, 0:D]).astype(bf16).T, u32)
    modr[0] = mod[:, D:2 * D]
    modr[1] = mod[:, 2 * D:3 * D] + 1.0
    toks += wo_res(0)
    attn(1, NG - 1)
    ln1(2, 2, 0, _Ticker(toks[20:240], N_LN1))

    for i in range(3, NA):
        cp_x(i).wait()

    def a_tile(i):
        toks = []
        for u in range(NG):
            toks += qkv_part(i, u)
            if u > 0:
                attn(i, u - 1)
        h2 = ln2a(i - 2, notick)
        toks += wo_res(i - 1)
        attn(i, NG - 1)
        ln2b(i - 2, h2, _Ticker(toks[20:108] + toks[490:570], N_LN2B))
        ln1(jnp.minimum(_iv(i) + 1, NA - 1), jnp.minimum(_iv(i), NA - 2) + 1, (i + 1) % 2,
            _Ticker(toks[120:490], N_LN1))

    def a_body(it, carry):
        for d in range(2):
            a_tile(_Idx(2 + 2 * it, d))
        return carry

    jax.lax.fori_loop(0, (NA - 2) // 2, a_body, 0)

    cp_modc.wait()
    for j in range(NF):
        for k in range(3):
            cp_f(k, j).wait()
    modb[2] = col_bcast(mod_cols(MOD_B - L, 6 * D)[:, 5 * D - (MOD_B - L):])
    toks = wo_res(NA - 1)
    ln2b(NA - 2, ln2a(NA - 2, notick), _Ticker(toks[0:100], N_LN2B))

    def fin(ii, ri, tk):
        cs = slice(ii * L, (ii + 1) * L)
        cc = _hk_c_row(lambda k: acc[k, :, cs], ri, _ticks(tk, QD // 8))
        if 2 * ii < UNITS[1][0]:
            lo = jax.lax.broadcasted_iota(jnp.int32, (QD, L), 1) < 64
            for a1 in range(2):
                v0, v1 = cc[2 * a1], cc[2 * a1 + 1]
                z = pltpu.roll(jnp.where(lo, v1, v0), 64, 1)
                cc[2 * a1], cc[2 * a1 + 1] = jnp.where(lo, v0, z), jnp.where(lo, z, v1)
        rows = slice(ri * QD, (ri + 1) * QD)
        out_v[ii, rows, :] = jnp.concatenate(
            [x1_sc[4 * ii + 2 * par + a1, rows] + modb[2, rows] * cc[2 * a1 + par] for par, a1 in QS],
            axis=1).astype(bf16)

    def b_body(j, carry):
        js = (j, jnp.minimum(j, NF - 1), jnp.maximum(j, 0), jnp.clip(j, 0, NF - 1))
        bw = {}
        for c1, wv in enumerate((w1_v, w3_v)):
            for a in SORD:
                jj = js[(0, 1, 1, 2, 2, 3, 3)[a]]
                blk = lambda p: wv[jj, 256 * p[0]:256 * p[0] + 256, HF * p[1]:HF * p[1] + HF].astype(f32)
                p0, p1, sgn = SRIN[a]
                y = blk(p0) if p1 is None else blk(p0) + blk(p1) if sgn > 0 else blk(p0) - blk(p1)
                for b, v in enumerate(_sb(y[0:L, 0:L], y[0:L, L:], y[L:, 0:L], y[L:, L:])):
                    bw[(c1, a, b)] = v.astype(bf16)
        aw = [v.astype(bf16) for v in _hk_a(lambda l, i: (
            w2t_v[js[l], i * QD:(i + 1) * QD, 0:HF].astype(f32),
            w2t_v[js[l], i * QD:(i + 1) * QD, HF:TF].astype(f32)))]

        def gate_up(tt):
            t0, nt = UNITS[tt]
            rq = slice(t0 * 32, (t0 + nt) * 32)
            main, rem = {}, {}
            for c1 in range(2):
                for a in SORD:
                    for b in SORD:
                        main[(c1, a, b)] = jnp.dot(_upk(a_sc[7 * a + b, rq, :]), bw[(c1, a, b)],
                                                   preferred_element_type=f32)
            for a1, a2 in QS:
                for c2, nn in QS:
                    for c1, wv in enumerate((w1_v, w3_v)):
                        col = c2 * HF + nn * L
                        rem[(c1, a1, c2, a2, nn)] = jnp.dot(
                            _upk(t_sc[2 * a1 + a2, rq, :]), wv[j, 512:D, col:col + L],
                            preferred_element_type=f32)
            keep = lambda v: jnp.concatenate([v[0:64], v[64:]], axis=0)
            g, u = [_strassen_out(lambda a, b: keep(main[(c1, a, b)]),
                                  {k1 + k2: keep(rem[(c1,) + k1 + k2]) for k1 in QS for k2 in QS})
                    for c1 in range(2)]
            act = {k: _silu_mul(g[k], u[k]) for k in g}

            def blk(a1, y, c2):
                if tt == 0:
                    return jnp.concatenate([act[(a1, c2, y, nn)] for nn in range(2)], axis=1)
                return jnp.concatenate([
                    jnp.concatenate([act[(a1, c2, a2, nn)][64 * tl:64 * tl + 64]
                                     for tl in range(y, nt, 2) for a2 in range(2)], axis=0)
                    for nn in range(2)], axis=1)

            eb = [v.astype(bf16) for v in _hk_b([blk(a1, a2, 0) for a1, a2 in QS],
                                                [blk(a1, a2, 1) for a1, a2 in QS])]
            return eb, list(main.values())

        def down(tt, eb):
            t0, nt = UNITS[tt]
            res = []
            for k in DORD:
                d = jax.lax.dot_general(aw[k], eb[k], NT, preferred_element_type=f32)
                acc[k, :, t0 * 64:(t0 + nt) * 64] += d
                res.append(d)
            return res

        def finish(tt, prods):
            t0, nt = UNITS[tt]
            toks = [t for v in prods for t in _toks(v, 16, L)]
            tk = _Ticker(toks, 2 * nt * (QD // 8))
            for ii in range(t0 // 2, (t0 + nt) // 2):
                for ri in range(4):
                    fin(ii, ri, tk)

                    @pl.when(j == NF - 1)
                    def _():
                        cp_o(ii, ri).start()

        eb0, _ = gate_up(0)
        eb1, prods = gate_up(1)
        gt = [t for v in prods for t in _toks(v, 32)]
        n = len(gt)
        ln2b(NA - 1, ln2a(NA - 1, _Ticker(gt[n * 8 // 100:n * 32 // 100], N_LN2A)),
             _Ticker(gt[n * 35 // 100:n * 95 // 100], N_LN2B))
        down(0, eb0)
        eb2, prods = gate_up(2)
        finish(0, prods[0:92])
        down(1, eb1)
        finish(1, down(2, eb2)[0:20])
        return carry

    jax.lax.fori_loop(0, NF, b_body, 0)

    for ri in range(4):
        fin(NA // 2 - 1, ri, notick)
        cp_o(NA // 2 - 1, ri).start()
    for ii in range(NA // 2):
        for ri in range(4):
            cp_o(ii, ri).wait()


@jax.jit
def pallas_adaLN_cond__sliding_local_dilated__glu_gated_swiglu__prompt_kernel(
    A_x: jax.Array,
    A_wqkv: jax.Array,
    A_wo: jax.Array,
    B_x: jax.Array,
    B_w1: jax.Array,
    B_w3: jax.Array,
    B_w2: jax.Array,
    c: jax.Array,
    w_mod: jax.Array,
):
    del B_x
    hbm = pl.BlockSpec(memory_space=pl.ANY)
    out_t = pl.pallas_call(
        _kernel,
        in_specs=[hbm] * 8,
        out_specs=hbm,
        out_shape=jax.ShapeDtypeStruct((D, S), bf16),
        scratch_shapes=[
            pltpu.VMEM((1, D), bf16),
            pltpu.VMEM((NA, D, TA), bf16),
            pltpu.VMEM((D, 6 * D), bf16),
            pltpu.VMEM((D, 3 * D), bf16),
            pltpu.VMEM((3 * D // 2, D), u32),
            pltpu.VMEM((D, D), bf16),
            pltpu.VMEM((D // 2, D), u32),
            pltpu.VMEM((NF, D, TF), bf16),
            pltpu.VMEM((NF, D, TF), bf16),
            pltpu.VMEM((NF, D, TF), bf16),
            pltpu.VMEM((3, D, L), f32),
            pltpu.VMEM((2, 8, D), f32),
            pltpu.VMEM((2, D // 2, TA), u32),
            pltpu.VMEM((2, NG, HR, L), f32),
            pltpu.VMEM((2 * NA + 1, NG, HR // 2, L), u32),
            pltpu.VMEM((2 * NA + 1, NG, HR, L), f32),
            pltpu.VMEM((2, 2, D, L), f32),
            pltpu.VMEM((2 * NA, D, L), f32),
            pltpu.VMEM((NA, 3, 8, TA), f32),
            pltpu.VMEM((49, S // 8, L), u32),
            pltpu.VMEM((4, S // 8, 64), u32),
            pltpu.VMEM((26, QD, S // 4), f32),
            pltpu.VMEM((NA // 2, D, 2 * TA), bf16),
            pltpu.SemaphoreType.DMA((6,)),
        ],
        compiler_params=pltpu.CompilerParams(vmem_limit_bytes=100 * 1024 * 1024),
    )(A_x.reshape(S, D).T, c, w_mod, A_wqkv, A_wo, B_w1, B_w3, B_w2.T)
    return out_t.T.reshape(1, S, D)
```
